```python
import os as _os
_os.environ.setdefault("JAX_PLATFORMS", "cpu")
import jax
import jax.numpy as jnp

def _softmax(x, axis=-1):
    return jax.nn.softmax(x, axis=axis)
def _gelu(x):
    return jax.nn.gelu(x, approximate=True)
def _silu(x):
    return jax.nn.silu(x)
def _sigmoid(x):
    return jax.nn.sigmoid(x)
def _layernorm(x, axis=-1, eps=1e-5):
    m = jnp.mean(x, axis=axis, keepdims=True)
    v = jnp.var(x, axis=axis, keepdims=True)
    return (x - m) / jnp.sqrt(v + eps)
def _scatter_add(tgt, idx, src, axis=0):
    return tgt.at[idx].add(src)
def _segment_sum(src, seg, n):
    return jax.ops.segment_sum(src, seg, n)
class _Rng:
    def __init__(self, key):
        self._k = key
    def _next(self):
        self._k, sub = jax.random.split(self._k)
        return sub
    def normal(self, shape):
        return jax.random.normal(self._next(), shape, dtype=jnp.bfloat16)
    def randint(self, lo, hi, shape):
        return jax.random.randint(self._next(), shape, lo, hi, dtype=jnp.int32)
    def uniform(self, shape, lo=0.0, hi=1.0):
        return jax.random.uniform(self._next(), shape, jnp.bfloat16, lo, hi)
    def permutation(self, n):
        return jax.random.permutation(self._next(), n)


kernel_name = 'gated_mix__linear_kernel_hedgehog__mixer_s_mlp__prompt'

def setup_inputs():
    _rng = _Rng(jax.random.key(int.from_bytes(__import__("os").urandom(4), "little")))
    _w = (lambda a: (lambda t: t.astype(jnp.bfloat16) if jnp.issubdtype(t.dtype, jnp.floating) else t)(jnp.asarray(a)))
    def _A_setup():
        B, S, D, H = 1, 2048, 512, 32
        Dh = D // H
        return {
            "x": _w((lambda *s: _rng.normal(s) * 0.05)(B, S, D)),
            "wqkv": _w((lambda *s: _rng.normal(s) * 1.6)(D, 3 * D)),
            "w_phi": _w((lambda *s: _rng.normal(s) * 1.6)(H, Dh, Dh) * (Dh ** -0.5)),
            "wo": _w((lambda *s: _rng.normal(s) * 0.05)(D, D)),
        }
    _A_in = _A_setup()

    def _B_setup():
        B, S, D, F = 1, 2048, 512, 1376
        return {
            "x":  _w((lambda *s: _rng.normal(s) * 0.05)(B, S, D)),
            "w1": _w((lambda *s: _rng.normal(s) * 0.4)(D, D) * (D ** -0.5)),
            "w2": _w((lambda *s: _rng.normal(s) * 0.4)(D, D) * (D ** -0.5)),
            "w3": _w((lambda *s: _rng.normal(s) * 0.4)(D, F) * (D ** -0.5)),
            "w4": _w((lambda *s: _rng.normal(s) * 0.4)(F, D) * (F ** -0.5)),
        }
    _B_in = _B_setup()

    return {
        "A_x": _A_in["x"],
        "A_wqkv": _A_in["wqkv"],
        "A_w_phi": _A_in["w_phi"],
        "A_wo": _A_in["wo"],
        "B_x": _B_in["x"],
        "B_w1": _B_in["w1"],
        "B_w2": _B_in["w2"],
        "B_w3": _B_in["w3"],
        "B_w4": _B_in["w4"],
        "gate_w": _w((lambda *s: _rng.normal(s) * 0.05)(512) * 16.0),
    }

def reference(A_x, A_wqkv, A_w_phi, A_wo, B_x, B_w1, B_w2, B_w3, B_w4, gate_w):
    def _A_ref(x, wqkv, w_phi, wo):
        B, S, D = x.shape
        H = 32; Dh = D // H
        qkv = (lambda x, *d: x.transpose(*d))((x @ wqkv).reshape(B, S, 3, H, Dh), 2, 0, 3, 1, 4)
        q, k, v = qkv[0], qkv[1], qkv[2]
        pq = jnp.einsum("bhsd,hdf->bhsf", q, w_phi)
        pk = jnp.einsum("bhsd,hdf->bhsf", k, w_phi)
        phi_q = jnp.concatenate([_softmax(pq, axis=-1), _softmax(-pq, axis=-1)], axis=-1)
        phi_k = jnp.concatenate([_softmax(pk, axis=-1), _softmax(-pk, axis=-1)], axis=-1)
        kv = jnp.einsum("bhsf,bhsd->bhfd", phi_k, v)
        z  = jnp.einsum("bhsf->bhf", phi_k)
        num = jnp.einsum("bhqf,bhfd->bhqd", phi_q, kv)
        den = jnp.einsum("bhqf,bhf->bhq", phi_q, z)[..., None] + 1e-6
        o = num / den
        return (lambda x, *d: x.transpose(*d))(o, 0, 2, 1, 3).reshape(B, S, D) @ wo

    def _B_ref(x, w1, w2, w3, w4):
        B, S, D = x.shape
        h = _gelu(_layernorm(x, axis=-1) @ w1)
        c = D // 4
        g0 = jnp.pad(h[:, :, 0*c:1*c], ((0, 0), (1, 0), (0, 0)))[:, :S, :]
        g1 = jnp.pad(h[:, :, 1*c:2*c], ((0, 0), (0, 1), (0, 0)))[:, 1:, :]
        g2 = jnp.pad(h[:, :, 2*c:3*c], ((0, 0), (2, 0), (0, 0)))[:, :S, :]
        g3 = jnp.pad(h[:, :, 3*c:   ], ((0, 0), (0, 2), (0, 0)))[:, 2:, :]
        hs = jnp.concatenate([g0, g1, g2, g3], axis=-1) @ w2
        x1 = x + hs
        h2 = _gelu(_layernorm(x1, axis=-1) @ w3) @ w4
        return x1 + h2

    x = A_x
    g = _sigmoid((x * gate_w).sum(-1, keepdims=True))
    a = _A_ref(x, A_wqkv, A_w_phi, A_wo)
    b = _B_ref(x, B_w1, B_w2, B_w3, B_w4)
    return g * a + (1 - g) * b
```

```python
import functools
import jax
import jax.numpy as jnp
from jax import lax
import jax.experimental.pallas as pl
import jax.experimental.pallas.tpu as pltpu

F32 = jnp.float32
BF16 = jnp.bfloat16
TM1 = 256
TM2 = 256
UNROLL = 0
NT_DIMS = (((1,), (1,)), ((), ()))
TN_DIMS = (((0,), (0,)), ((), ()))


def _gelu(x):
    c = 0.7978845608028654
    return 0.5 * x * (1.0 + jnp.tanh(c * (x + 0.044715 * (x * x * x))))


def _ln(xf):
    m = jnp.mean(xf, axis=-1, keepdims=True)
    xc = xf - m
    v = jnp.mean(xc * xc, axis=-1, keepdims=True)
    return xc * lax.rsqrt(v + 1e-5)


def _fold4(a, op):
    return op(a, pltpu.roll(a, 4, 0))


def _exps(p, tm):
    p3 = p.reshape(8, 8, tm)
    mx = _fold4(jnp.max(p3, axis=0), jnp.maximum)
    mn = _fold4(jnp.min(p3, axis=0), jnp.minimum)
    ep = jnp.exp(p3 - mx[None])
    en = jnp.exp(mn[None] - p3)
    sp = _fold4(jnp.sum(ep, axis=0), jnp.add)
    sn = _fold4(jnp.sum(en, axis=0), jnp.add)
    return ep, en, sp, sn


def _kernel(x_hbm, wqkv_hbm, wphi_hbm, wo_hbm, w1_hbm, w2_hbm, w3t_hbm, w4_hbm, gw_hbm,
            out_hbm,
            x_v, wqkv_v, wphi_v, wo_v, w1_v, w2_v, w3t_v, w4_v, gw_v, o_v,
            p_s, wkvT, wqT, h_scr, kv_acc, z_acc, kvT, zb, sems, osems,
            *, S, D, tm1, tm2):
    n1 = S // tm1
    n2 = S // tm2

    def cp(src, dst, k):
        return pltpu.make_async_copy(src, dst, sems.at[k])

    c_phi = cp(wphi_hbm, wphi_v, 0)
    c_x0 = cp(x_hbm.at[pl.ds(0, tm1)], x_v.at[pl.ds(0, tm1)], 1)
    c_w1 = cp(w1_hbm, w1_v, 2)
    c_kv = cp(wqkv_hbm.at[:, pl.ds(D, 2 * D)], wqkv_v.at[:, pl.ds(D, 2 * D)], 3)
    c_xr = cp(x_hbm.at[pl.ds(tm1, S - tm1)], x_v.at[pl.ds(tm1, S - tm1)], 4)
    c_q = cp(wqkv_hbm.at[:, pl.ds(0, D)], wqkv_v.at[:, pl.ds(0, D)], 5)
    c_gw = cp(gw_hbm, gw_v, 6)
    c_w2 = cp(w2_hbm, w2_v, 7)
    c_w3 = cp(w3t_hbm, w3t_v, 8)
    c_w4 = cp(w4_hbm, w4_v, 9)
    c_wo = cp(wo_hbm, wo_v, 10)
    for c in (c_phi, c_x0, c_w1, c_kv, c_xr, c_q, c_gw, c_w2, c_w3, c_w4, c_wo):
        c.start()

    kv_acc[...] = jnp.zeros_like(kv_acc)
    z_acc[...] = jnp.zeros_like(z_acc)
    h_scr[:, 0:8, :] = jnp.zeros((4, 8, 128), F32)
    h_scr[:, S + 8:S + 16, :] = jnp.zeros((4, 8, 128), F32)

    c_phi.wait()
    r = lax.broadcasted_iota(jnp.int32, (D, 32), 0)
    c = lax.broadcasted_iota(jnp.int32, (D, 32), 1)
    A = (((r // 64) * 4 + r % 4) == c).astype(BF16)
    T1 = lax.dot_general(A, wphi_v[...], NT_DIMS, preferred_element_type=F32)
    r = lax.broadcasted_iota(jnp.int32, (D, 256), 0)
    c = lax.broadcasted_iota(jnp.int32, (D, 256), 1)
    T2 = jnp.where(((r // 4) % 16) == (c % 16), T1, 0.0).astype(BF16)
    r = lax.broadcasted_iota(jnp.int32, (256, 128), 0)
    c = lax.broadcasted_iota(jnp.int32, (256, 128), 1)
    Bm = ((r // 16) == (c % 16)).astype(BF16)
    P = jnp.dot(T2, Bm, preferred_element_type=F32)
    r = lax.broadcasted_iota(jnp.int32, (D, 128), 0)
    c = lax.broadcasted_iota(jnp.int32, (D, 128), 1)
    p_s[...] = jnp.where((((r // 64) % 2) * 4 + r % 4) == (c // 16), P, 0.0).astype(BF16)

    def fold(dst, row0, col0):
        for hg in range(4):
            W = wqkv_v[:, col0 + hg * 128: col0 + (hg + 1) * 128]
            WT = lax.dot_general(p_s[hg * 128:(hg + 1) * 128, :], W, NT_DIMS,
                                 preferred_element_type=F32)
            dst[row0 + hg * 128: row0 + (hg + 1) * 128, :] = WT.astype(BF16)

    def b1(r0, tm):
        x = x_v[pl.ds(r0, tm), :]
        ln = _ln(x.astype(F32)).astype(BF16)
        h = _gelu(jnp.dot(ln, w1_v[...], preferred_element_type=F32))
        for g in range(4):
            h_scr[g, pl.ds(r0 + 8, tm), :] = h[:, g * 128:(g + 1) * 128]

    def a1(r0, tm, mid):
        x = x_v[pl.ds(r0, tm), :]
        kvp = lax.dot_general(wkvT[...], x, NT_DIMS, preferred_element_type=F32)
        mid()
        for g in range(8):
            ep, en, sp, sn = _exps(kvp[g * 64:(g + 1) * 64, :], tm)
            fk = jnp.concatenate([(ep * (1.0 / sp)[None]).reshape(64, tm),
                                  (en * (1.0 / sn)[None]).reshape(64, tm)], axis=0)
            zs = fk[:, 0:128]
            for t in range(1, tm // 128):
                zs = zs + fk[:, t * 128:(t + 1) * 128]
            z_acc[g] += zs
            vT = kvp[D + g * 64: D + (g + 1) * 64, :].astype(BF16)
            kv_acc[g] += lax.dot_general(vT, fk.astype(BF16), NT_DIMS,
                                         preferred_element_type=F32)

    c_x0.wait()
    c_w1.wait()
    b1(0, tm1)
    c_kv.wait()
    fold(wkvT, 0, D)
    wkvT[D:2 * D, :] = wqkv_v[:, 2 * D:3 * D].T
    a1(0, tm1, lambda: None)
    c_xr.wait()

    def p1(i, carry):
        r0 = i * tm1 if isinstance(i, int) else pl.multiple_of(i * tm1, tm1)
        a1(r0, tm1, lambda: b1(r0, tm1))
        return carry

    if UNROLL:
        for i in range(1, n1):
            p1(i, 0)
    else:
        lax.fori_loop(1, n1, p1, 0)

    c_q.wait()
    fold(wqT, 0, 0)
    r = lax.broadcasted_iota(jnp.int32, (64, 128), 0)
    c = lax.broadcasted_iota(jnp.int32, (64, 128), 1)
    msk = (r // 16) == (c % 4)
    for g in range(8):
        kvT[g] = jnp.where(msk, kv_acc[g], 0.0).astype(BF16)
        zb[g] = jnp.broadcast_to(jnp.sum(z_acc[g], axis=1, keepdims=True), (128, 128))
    c_gw.wait()
    c_w2.wait()
    c_w3.wait()
    c_w4.wait()
    c_wo.wait()

    def p2(j, carry):
        tm = tm2
        r0 = j * tm if isinstance(j, int) else pl.multiple_of(j * tm, tm)
        x = x_v[pl.ds(r0, tm), :]
        xf = x.astype(F32)
        shifts = (-1, 1, -2, 2)
        hsft = jnp.concatenate(
            [h_scr[g, pl.ds(r0 + 8 + shifts[g], tm), :] for g in range(4)], axis=1).astype(BF16)
        x1 = xf + jnp.dot(hsft, w2_v[...], preferred_element_type=F32)
        qT = lax.dot_general(wqT[...], x, NT_DIMS, preferred_element_type=F32)
        ln2 = _ln(x1).astype(BF16)
        h3 = _gelu(lax.dot_general(ln2, w3t_v[...], NT_DIMS,
                                   preferred_element_type=F32)).astype(BF16)
        oTs = []
        for g in range(8):
            ep, en, sp, sn = _exps(qT[g * 64:(g + 1) * 64, :], tm)
            z = zb[g]
            zt = jnp.concatenate([z] * (tm // 128), axis=1)
            ap = _fold4(jnp.sum(ep * zt[0:64].reshape(8, 8, tm), axis=0), jnp.add)
            an = _fold4(jnp.sum(en * zt[64:128].reshape(8, 8, tm), axis=0), jnp.add)
            rp = 1.0 / sp
            rn = 1.0 / sn
            rden = 1.0 / (ap * rp + an * rn + 1e-6)
            fq = jnp.concatenate([(ep * (rp * rden)[None]).reshape(64, tm),
                                  (en * (rn * rden)[None]).reshape(64, tm)], axis=0)
            oTs.append(jnp.dot(kvT[g], fq.astype(BF16), preferred_element_type=F32).astype(BF16))
        oT = jnp.concatenate(oTs, axis=0)
        b = x1 + jnp.dot(h3, w4_v[...], preferred_element_type=F32)
        a = lax.dot_general(oT, wo_v[...], TN_DIMS, preferred_element_type=F32)
        gw = gw_v[...].astype(F32)
        gs = xf[:, 0:128] * gw[0:1]
        for g in range(1, 4):
            gs = gs + xf[:, g * 128:(g + 1) * 128] * gw[g:g + 1]
        gate = jax.nn.sigmoid(jnp.sum(gs, axis=-1, keepdims=True))
        o_v[pl.ds(r0, tm), :] = (gate * a + (1.0 - gate) * b).astype(BF16)
        pltpu.make_async_copy(o_v.at[pl.ds(r0, tm)], out_hbm.at[pl.ds(r0, tm)],
                              osems.at[j]).start()
        return carry

    if UNROLL:
        for j in range(n2):
            p2(j, 0)
    else:
        lax.fori_loop(0, n2, p2, 0)

    for j in range(n2):
        pltpu.make_async_copy(o_v.at[pl.ds(j * tm2, tm2)], out_hbm.at[pl.ds(j * tm2, tm2)],
                              osems.at[j]).wait()


@jax.jit
def pallas_gated_mix__linear_kernel_hedgehog__mixer_s_mlp__prompt_kernel(
    A_x, A_wqkv, A_w_phi, A_wo, B_x, B_w1, B_w2, B_w3, B_w4, gate_w):
    B, S, D = A_x.shape
    Fd = B_w3.shape[1]
    x2 = A_x.reshape(S, D)
    wphi2 = A_w_phi.transpose(1, 2, 0).reshape(256, 32)
    gw2 = gate_w.reshape(4, 128)
    w3t = B_w3.T
    anyspec = pl.BlockSpec(memory_space=pl.ANY)
    out = pl.pallas_call(
        functools.partial(_kernel, S=S, D=D, tm1=TM1, tm2=TM2),
        in_specs=[anyspec] * 9,
        out_specs=anyspec,
        out_shape=jax.ShapeDtypeStruct((S, D), A_x.dtype),
        scratch_shapes=[
            pltpu.VMEM((S, D), BF16),
            pltpu.VMEM((D, 3 * D), BF16),
            pltpu.VMEM((256, 32), BF16),
            pltpu.VMEM((D, D), BF16),
            pltpu.VMEM((D, D), BF16),
            pltpu.VMEM((D, D), BF16),
            pltpu.VMEM((Fd, D), BF16),
            pltpu.VMEM((Fd, D), BF16),
            pltpu.VMEM((4, 128), BF16),
            pltpu.VMEM((S, D), BF16),
            pltpu.VMEM((D, 128), BF16),
            pltpu.VMEM((2 * D, D), BF16),
            pltpu.VMEM((D, D), BF16),
            pltpu.VMEM((4, S + 16, 128), F32),
            pltpu.VMEM((8, 64, 128), F32),
            pltpu.VMEM((8, 128, 128), F32),
            pltpu.VMEM((8, 64, 128), BF16),
            pltpu.VMEM((8, 128, 128), F32),
            pltpu.SemaphoreType.DMA((11,)),
            pltpu.SemaphoreType.DMA((S // TM2,)),
        ],
        compiler_params=pltpu.CompilerParams(vmem_limit_bytes=100 * 1024 * 1024),
    )(x2, A_wqkv, wphi2, A_wo, B_w1, B_w2, w3t, B_w4, gw2)
    return out.reshape(B, S, D)
```

```python
import functools
import jax
import jax.numpy as jnp
from jax import lax
import jax.experimental.pallas as pl
import jax.experimental.pallas.tpu as pltpu

F32 = jnp.float32
BF16 = jnp.bfloat16
U32 = jnp.uint32
TM = 256
U2 = 4
SCOPES = 0
ZMX = 0
REM = 1
R5 = 'a'
NT_DIMS = (((1,), (1,)), ((), ()))
TN_DIMS = (((0,), (0,)), ((), ()))
GC = 0.7978845608028654
LOG2E = 1.4426950408889634


def _gelu(x):
    return (0.5 * x) * (1.0 + jnp.tanh(x * (GC + (GC * 0.044715) * (x * x))))


def _rcp(x):
    return pl.reciprocal(x, approx=False, full_range=False)


def _ln_stats(xf):
    m = jnp.mean(xf, axis=-1, keepdims=True)
    v = jnp.maximum(jnp.mean(xf * xf, axis=-1, keepdims=True) - m * m, 0.0)
    return m, lax.rsqrt(v + 1e-5)


def _pk(x):
    return pltpu.bitcast(x.astype(BF16), U32)


def _up(x):
    return pltpu.bitcast(x, BF16)


def _fold4(a, op):
    return op(a, pltpu.roll(a, 4, 0))


def _exps(p, tm):
    p3 = p.reshape(8, 8, tm)
    mx = _fold4(jnp.max(p3, axis=0), jnp.maximum)
    mn = _fold4(jnp.min(p3, axis=0), jnp.minimum)
    ep = jnp.exp2(p3 - mx[None])
    en = jnp.exp2(mn[None] - p3)
    sp = _fold4(jnp.sum(ep, axis=0), jnp.add)
    sn = _fold4(jnp.sum(en, axis=0), jnp.add)
    return ep, en, sp, sn


def _kernel(x_hbm, wqkv_hbm, wphi_hbm, wo_hbm, w1_hbm, w2_hbm, w3t_hbm, w4_hbm, gw_hbm,
            out_hbm,
            x_v, wqkv_v, wphi_v, wo_v, w1_v, w2_v, w3t_v, w4_v, gw_v, o_v,
            p_s, wkT, wvT, wqT, h_scr, kvT, zb, g_s, ng_s, sems,
            *, S, D, Fd, tm):
    nt = S // tm
    _cur = []

    def sc(name):
        if not SCOPES:
            return
        if _cur:
            _cur.pop().__exit__(None, None, None)
        if name:
            c_ = jax.named_scope(name)
            c_.__enter__()
            _cur.append(c_)

    def cp(src, dst, k):
        return pltpu.make_async_copy(src, dst, sems.at[k])

    def cols(k):
        return (slice(None), pl.ds(k * D, D))

    def rows(a, n):
        return pl.ds(a * tm, n * tm)

    copies = [
        [cp(wphi_hbm, wphi_v, 0), cp(gw_hbm, gw_v, 0)],
        [cp(wqkv_hbm.at[cols(1)], wqkv_v.at[cols(1)], 1)],
        [cp(x_hbm.at[rows(0, 1)], x_v.at[rows(0, 1)], 2)],
        [cp(w1_hbm, w1_v, 3)],
        [cp(x_hbm.at[rows(1, 1)], x_v.at[rows(1, 1)], 4),
         cp(wqkv_hbm.at[cols(2)], wqkv_v.at[cols(2)], 4)],
        [cp(x_hbm.at[rows(2, nt - 2)], x_v.at[rows(2, nt - 2)], 5),
         cp(wqkv_hbm.at[cols(0)], wqkv_v.at[cols(0)], 5)],
        [cp(w2_hbm, w2_v, 6), cp(w3t_hbm, w3t_v, 6), cp(w4_hbm, w4_v, 6), cp(wo_hbm, wo_v, 6)],
    ]
    sc('r0')
    for grp in copies:
        for c in grp:
            c.start()

    def wait(k):
        sc('w%d' % k)
        for c in copies[k]:
            c.wait()
        sc('r%d' % (k + 1))

    h_scr[:, 0:8, :] = jnp.zeros((4, 8, 128), F32)
    h_scr[:, S + 8:S + 16, :] = jnp.zeros((4, 8, 128), F32)

    def row_info(n):
        rr = lax.broadcasted_iota(jnp.int32, (D, n), 0)
        hg = rr // 128
        rr = rr % 128
        f = jnp.where(rr < 16, rr // 8, jnp.where(rr < 72, rr // 4 - 2, rr // 4 - 16))
        hl8 = jnp.where(rr < 16, rr % 8, jnp.where(rr < 72, rr % 4, 4 + rr % 4))
        return hg, f, hl8, lax.broadcasted_iota(jnp.int32, (D, n), 1)

    wait(0)
    hg_, f_, hl8_, c = row_info(32)
    A = ((hg_ * 8 + hl8_) == c).astype(BF16)
    T1 = lax.dot_general(A, wphi_v[...], NT_DIMS, preferred_element_type=F32)
    hg_, f_, hl8_, c = row_info(256)
    T2 = jnp.where(f_ == (c % 16), T1, 0.0).astype(BF16)
    r = lax.broadcasted_iota(jnp.int32, (256, 128), 0)
    c = lax.broadcasted_iota(jnp.int32, (256, 128), 1)
    Bm = ((r // 16) == (c % 16)).astype(BF16)
    P = jnp.dot(T2, Bm, preferred_element_type=F32)
    hg_, f_, hl8_, c = row_info(128)
    p_s[...] = jnp.where(hl8_ == (c // 16), P, 0.0).astype(BF16)
    gw = gw_v[...].astype(F32)
    gwr = jnp.concatenate([gw[g:g + 1] for g in range(4)], axis=1)
    wkT[0:8, :] = _pk(jnp.broadcast_to(gwr, (16, D)))

    def fold(col0):
        lo = lax.broadcasted_iota(jnp.int32, (8, D), 0) < 4
        outs = []
        for hg in range(4):
            W = wqkv_v[:, col0 + hg * 128: col0 + (hg + 1) * 128]
            WT = lax.dot_general(p_s[hg * 128:(hg + 1) * 128, :], W, NT_DIMS,
                                 preferred_element_type=F32) * LOG2E
            ref = WT[0:8]
            rot = pltpu.roll(ref, 4, 0)
            outs.append(WT[8:16] - ref)
            outs.append((WT[16:72].reshape(7, 8, D) - jnp.where(lo, ref, rot)[None]).reshape(56, D))
            outs.append((WT[72:128].reshape(7, 8, D) - jnp.where(lo, rot, ref)[None]).reshape(56, D))
        return _pk(jnp.concatenate(outs, axis=0))

    def groups(pT):
        lo = lax.broadcasted_iota(jnp.int32, (8, tm), 0) < 4
        for hg in range(4):
            blk = pT[hg * 120:(hg + 1) * 120]
            mid = blk[0:8]
            yield jnp.concatenate([jnp.where(lo, mid, 0.0), blk[8:64]], axis=0)
            yield jnp.concatenate([jnp.where(lo, 0.0, mid), blk[64:120]], axis=0)

    def row0(j):
        return j * tm if isinstance(j, int) else pl.multiple_of(j * tm, tm)

    def xt(j):
        return x_v[pl.ds(row0(j), tm), :]

    cs = []

    def h_stage(j, stats):
        m, r = stats
        if not cs:
            lhs = jnp.concatenate([jnp.ones((16, D), BF16), xt(j)], axis=0)
            y = jnp.dot(lhs, w1_v[...], preferred_element_type=F32)
            cs.append(y[0:1])
            y = y[16:]
        else:
            y = jnp.dot(xt(j), w1_v[...], preferred_element_type=F32)
        h = _gelu((y - m * cs[0]) * r)
        for g in range(4):
            h_scr[g, pl.ds(row0(j) + 8, tm), :] = h[:, g * 128:(g + 1) * 128]

    def proj(w, j):
        return lax.dot_general(_up(w[...]), xt(j), NT_DIMS, preferred_element_type=F32)

    zs = [None] * 8
    kvs = [None] * 8

    def k_soft(j, kT):
        gate = jax.nn.sigmoid(kT[0:8])
        g_s[j] = gate
        ng_s[j] = jnp.concatenate([1.0 - gate] * 16, axis=0).T
        fks = []
        for g, pg in enumerate(groups(kT[16:496])):
            ep, en, sp, sn = _exps(pg, tm)
            fk = jnp.concatenate([(ep * _rcp(sp)[None]).reshape(64, tm),
                                  (en * _rcp(sn)[None]).reshape(64, tm)], axis=0)
            if not ZMX:
                part = fk[:, 0:128]
                for t in range(1, tm // 128):
                    part = part + fk[:, t * 128:(t + 1) * 128]
                zs[g] = part if zs[g] is None else zs[g] + part
            fks.append(fk.astype(BF16))
        return fks

    def v_split(vT):
        if ZMX:
            one = jnp.ones((16, tm), F32)
            return [jnp.concatenate([vT[g * 64:(g + 1) * 64, :], one], axis=0).astype(BF16)
                    for g in range(8)]
        return [vT[g * 64:(g + 1) * 64, :].astype(BF16) for g in range(8)]

    def kv_stage(fks, vT):
        for g in range(8):
            part = lax.dot_general(vT[g], fks[g], NT_DIMS, preferred_element_type=F32)
            if ZMX:
                part = part[0:72]
            kvs[g] = part if kvs[g] is None else kvs[g] + part

    def stats1(j):
        return _ln_stats(xt(j).astype(F32))

    wait(1)
    wkT[8:248, :] = fold(D)
    wait(2)
    kT0 = proj(wkT, 0)
    st0 = stats1(0)
    wait(3)
    h_stage(0, st0)
    wait(4)
    if R5 == 'a':
        kT1 = proj(wkT, 1)
        wvT[...] = _pk(wqkv_v[:, 2 * D:3 * D].T)
        fk0 = k_soft(0, kT0)
        v0 = v_split(proj(wvT, 0))
        fk1 = k_soft(1, kT1)
        v1 = v_split(proj(wvT, 1))
        kv_stage(fk0, v0)
        h_stage(1, stats1(1))
        kv_stage(fk1, v1)
    else:
        h_stage(1, stats1(1))
        wvT[...] = _pk(wqkv_v[:, 2 * D:3 * D].T)
        fk0 = k_soft(0, kT0)
        v0 = v_split(proj(wvT, 0))
        kT1 = proj(wkT, 1)
        kv_stage(fk0, v0)
        fk1 = k_soft(1, kT1)
        v1 = v_split(proj(wvT, 1))
        kv_stage(fk1, v1)
    wait(5)
    for j in range(2, nt):
        lhs = _up(jnp.concatenate(
            [wkT[0:128, :], wvT[0:128, :], wkT[128:248, :], wvT[128:256, :]], axis=0))
        pr = lax.dot_general(lhs, xt(j), NT_DIMS, preferred_element_type=F32)
        fk = k_soft(j, jnp.concatenate([pr[0:256], pr[512:752]], axis=0))
        vT = v_split(jnp.concatenate([pr[256:512], pr[752:1008]], axis=0))
        h_stage(j, stats1(j))
        if j == nt - 1 and not ZMX:
            for g in range(8):
                zb[g] = jnp.broadcast_to(jnp.sum(zs[g], axis=1, keepdims=True), (128, 128))
        kv_stage(fk, vT)
    wqT[...] = fold(0)
    r = lax.broadcasted_iota(jnp.int32, (64, 128), 0)
    c = lax.broadcasted_iota(jnp.int32, (64, 128), 1)
    msk = (r // 16) == (c % 4)
    for g in range(8):
        kvT[g] = _pk(jnp.where(msk, kvs[g][0:64], 0.0))
        if ZMX:
            zb[g] = jnp.concatenate([kvs[g][64:72]] * 16, axis=0).T

    wait(6)

    def w2_stage(j):
        r0 = row0(j)
        shifts = (-1, 1, -2, 2)
        hsft = jnp.concatenate(
            [h_scr[g, pl.ds(r0 + 8 + shifts[g], tm), :] for g in range(4)], axis=1).astype(BF16)
        x1 = xt(j).astype(F32) + jnp.dot(hsft, w2_v[...], preferred_element_type=F32)
        m, r = _ln_stats(x1)
        return x1, ((x1 - m) * r).astype(BF16)

    def q_stage(j):
        qT = proj(wqT, j)
        gate = g_s[j]
        fqs = []
        for g, pg in enumerate(groups(qT)):
            ep, en, sp, sn = _exps(pg, tm)
            z = zb[g]
            zt = jnp.concatenate([z] * (tm // 128), axis=1)
            ap = _fold4(jnp.sum(ep * zt[0:64].reshape(8, 8, tm), axis=0), jnp.add)
            an = _fold4(jnp.sum(en * zt[64:128].reshape(8, 8, tm), axis=0), jnp.add)
            rd = gate * _rcp(ap * sn + an * sp + 1e-6 * (sp * sn))
            fq = jnp.concatenate([(ep * (sn * rd)[None]).reshape(64, tm),
                                  (en * (sp * rd)[None]).reshape(64, tm)], axis=0)
            fqs.append(fq.astype(BF16))
        return fqs

    FM = (Fd // 128) * 128

    def w3_stage(ln2):
        if not REM:
            return _gelu(lax.dot_general(ln2, w3t_v[...], NT_DIMS,
                                         preferred_element_type=F32)).astype(BF16)
        hr = _gelu(lax.dot_general(w3t_v[FM:Fd, :], ln2, NT_DIMS,
                                   preferred_element_type=F32)).astype(BF16)
        hm = _gelu(lax.dot_general(ln2, w3t_v[0:FM, :], NT_DIMS,
                                   preferred_element_type=F32)).astype(BF16)
        return jnp.concatenate([hm, hr.T], axis=1)

    def num_stage(fqs):
        return jnp.concatenate(
            [jnp.dot(_up(kvT[g]), fqs[g], preferred_element_type=F32).astype(BF16)
             for g in range(8)], axis=0)

    def w4_stage(j, h3, x1):
        b = x1 + jnp.dot(h3, w4_v[...], preferred_element_type=F32)
        return b * jnp.concatenate([ng_s[j]] * 4, axis=1)

    def out_stage(j, oT, b, last):
        r0 = row0(j)
        o = oT.T
        for a0, n in ((0, 128), (128, 64), (192, 64)) if last else ((0, tm),):
            a = jnp.dot(o[a0:a0 + n], wo_v[...], preferred_element_type=F32)
            idx = pl.ds(r0 + a0, n)
            o_v[idx, :] = (a + b[a0:a0 + n]).astype(BF16)
            cp(o_v.at[idx], out_hbm.at[idx], 7).start()

    def body(j, x1, ln2, fqs, last):
        h3 = w3_stage(ln2)
        oT = num_stage(fqs)
        if not last:
            x1n, ln2n = w2_stage(j + 1)
        b = w4_stage(j, h3, x1)
        if not last:
            fqn = q_stage(j + 1)
        out_stage(j, oT, b, last)
        if not last:
            return x1n, ln2n, fqn

    def p2(i, carry):
        j0 = i * U2
        x1, ln2 = w2_stage(j0)
        fqs = q_stage(j0)
        st = (x1, ln2, fqs)
        for u in range(U2 - 1):
            st = body(j0 + u, *st, False)
        body(j0 + U2 - 1, *st, True)
        return carry

    lax.fori_loop(0, nt // U2, p2, 0)

    sc('w_out')
    cp(o_v, out_hbm, 7).wait()
    sc(None)


@jax.jit
def pallas_gated_mix__linear_kernel_hedgehog__mixer_s_mlp__prompt_kernel(
    A_x, A_wqkv, A_w_phi, A_wo, B_x, B_w1, B_w2, B_w3, B_w4, gate_w):
    B, S, D = A_x.shape
    Fd = B_w3.shape[1]
    x2 = A_x.reshape(S, D)
    wphi2 = A_w_phi.transpose(1, 2, 0).reshape(256, 32)
    gw2 = gate_w.reshape(4, 128)
    w3t = B_w3.T
    nt = S // TM
    anyspec = pl.BlockSpec(memory_space=pl.ANY)
    out = pl.pallas_call(
        functools.partial(_kernel, S=S, D=D, Fd=Fd, tm=TM),
        in_specs=[anyspec] * 9,
        out_specs=anyspec,
        out_shape=jax.ShapeDtypeStruct((S, D), A_x.dtype),
        scratch_shapes=[
            pltpu.VMEM((S, D), BF16),
            pltpu.VMEM((D, 3 * D), BF16),
            pltpu.VMEM((256, 32), BF16),
            pltpu.VMEM((D, D), BF16),
            pltpu.VMEM((D, D), BF16),
            pltpu.VMEM((D, D), BF16),
            pltpu.VMEM((Fd, D), BF16),
            pltpu.VMEM((Fd, D), BF16),
            pltpu.VMEM((4, 128), BF16),
            pltpu.VMEM((S, D), BF16),
            pltpu.VMEM((D, 128), BF16),
            pltpu.VMEM((248, D), U32),
            pltpu.VMEM((D // 2, D), U32),
            pltpu.VMEM((240, D), U32),
            pltpu.VMEM((4, S + 16, 128), F32),
            pltpu.VMEM((8, 32, 128), U32),
            pltpu.VMEM((8, 128, 128), F32),
            pltpu.VMEM((nt, 8, TM), F32),
            pltpu.VMEM((nt, TM, 128), F32),
            pltpu.SemaphoreType.DMA((8,)),
        ],
        compiler_params=pltpu.CompilerParams(vmem_limit_bytes=100 * 1024 * 1024,
                                             disable_bounds_checks=True),
    )(x2, A_wqkv, wphi2, A_wo, B_w1, B_w2, w3t, B_w4, gw2)
    return out.reshape(B, S, D)
```

```python
import functools
import jax
import jax.numpy as jnp
from jax import lax
import jax.experimental.pallas as pl
import jax.experimental.pallas.tpu as pltpu

F32 = jnp.float32
BF16 = jnp.bfloat16
U32 = jnp.uint32
T0 = 256
T1 = '256,256,256,256,256,256'
T2 = '256,256,256,256'
SW = '2o1v'
PAT2 = 'ccceeeqqebNeebO'
EARLY = '4'
SKIP = ''
ZMX = 0
PAT1 = 'K,v,v,v,v,h,h,a,a,a,a'
BAR = ''
HMAP = '012345'
GE = '01'
GL = '2345'
GG = 0
LINK = 0
PACE = '3'
NOCSE = 0
RF = 1
R5 = 'pKTsVthwAB'
P4 = 0
S3 = 1
PRO = 'bbqq'
C2 = 2
ZP = 'p1'
WPOS = 2
PRE = 'spread'
RB = 8
IL = 16
APX = 0
CH = '64,48,32,16'
NT_DIMS = (((1,), (1,)), ((), ()))
GC = 0.7978845608028654
LOG2E = 1.4426950408889634


def _gelu(x):
    return (0.5 * x) * (1.0 + jnp.tanh(x * (GC + (GC * 0.044715) * (x * x))))


def _rcp(x):
    return pl.reciprocal(x, approx=bool(APX), full_range=False)


def _ln_stats(xf):
    m = jnp.mean(xf, axis=-1, keepdims=True)
    v = jnp.maximum(jnp.mean(xf * xf, axis=-1, keepdims=True) - m * m, 0.0)
    return m, lax.rsqrt(v + 1e-5)


def _pk(x):
    return pltpu.bitcast(x.astype(BF16), U32)


def _up(x):
    return pltpu.bitcast(x, BF16)


def _fold4(a, op):
    return op(a, pltpu.roll(a, 4, 0))


def _exps(p):
    p3 = p.reshape(8, 8, p.shape[1])
    mx = _fold4(jnp.max(p3, axis=0), jnp.maximum)
    mn = _fold4(jnp.min(p3, axis=0), jnp.minimum)
    ep = jnp.exp2(p3 - mx[None])
    en = jnp.exp2(mn[None] - p3)
    sp = _fold4(jnp.sum(ep, axis=0), jnp.add)
    sn = _fold4(jnp.sum(en, axis=0), jnp.add)
    return ep, en, sp, sn


def _groups(pT):
    lo = lax.broadcasted_iota(jnp.int32, (8, pT.shape[1]), 0) < 4
    for hg in range(4):
        blk = pT[hg * 120:(hg + 1) * 120]
        mid = blk[0:8]
        yield jnp.concatenate([jnp.where(lo, mid, 0.0), blk[8:64]], axis=0)
        yield jnp.concatenate([jnp.where(lo, 0.0, mid), blk[64:120]], axis=0)


def _wino_a(a11, a12, a21, a22):
    s1 = a21 + a22
    s2 = s1 - a11
    s3 = a11 - a21
    s4 = a12 - s2
    return a11, a12, s4, a22, s1, s2, s3


def _split_rows(a):
    m, n = a.shape
    il = IL or m // 2
    a4 = a.reshape(m // (2 * il), 2, il, n)
    return a4[:, 0].reshape(m // 2, n), a4[:, 1].reshape(m // 2, n)


def _merge_rows(top, bot):
    h, n = top.shape
    il = IL or h
    return jnp.stack([top.reshape(h // il, il, n), bot.reshape(h // il, il, n)],
                     axis=1).reshape(2 * h, n)


def _wino_b(b11, b12, b21, b22):
    t1 = b12 - b11
    t2 = b22 - t1
    t3 = b22 - b12
    t4 = t2 - b21
    return t1, t2, t3, t4


def _wino_c(mm, a, b11, b21, b22, t1, t2, t3, t4):
    a11, a12, s4, a22, s1, s2, s3 = a
    p1 = mm(a11, b11)
    u2 = p1 + mm(s2, t2)
    c11 = p1 + mm(a12, b21)
    u3 = u2 + mm(s3, t3)
    p5 = mm(s1, t1)
    c12 = u2 + p5 + mm(s4, b22)
    c22 = u3 + p5
    c21 = u3 - mm(a22, t4)
    return c11, c12, c21, c22


TRACE = []


def _wino_gen(mm, a, b11, b21, b22, t1, t2, t3, t4):
    a11, a12, s4, a22, s1, s2, s3 = a
    p1 = mm(a11, b11)
    u2 = p1 + mm(s2, t2)
    TRACE.append(u2)
    yield None
    c11 = p1 + mm(a12, b21)
    u3 = u2 + mm(s3, t3)
    TRACE.append(u3)
    yield None
    p5 = mm(s1, t1)
    c12 = u2 + p5 + mm(s4, b22)
    c22 = u3 + p5
    TRACE.append(c12)
    yield None
    c21 = u3 - mm(a22, t4)
    yield c11, c12, c21, c22


def _nt(a, b):
    return lax.dot_general(a, b, NT_DIMS, preferred_element_type=F32)


def _nn(a, b):
    return jnp.dot(a, b, preferred_element_type=F32)


def _tiles(spec, start):
    out = []
    for t in spec.split(','):
        out.append((start, int(t)))
        start += int(t)
    return out


def _kernel(x_hbm, wqkv_hbm, wphi_hbm, wo_hbm, w1_hbm, w2_hbm, w3t_hbm, w4_hbm, gw_hbm,
            out_hbm,
            x_v, wqkv_v, wphi_v, w1_v, sv_s, wf_v, gw_v, o_v,
            p_s, wkT, wvT, wqT, h_scr, kvT, zb, z_s, g_s, ng_s, bar_v, sems,
            *, S, D, Fd):
    FM = (Fd // 256) * 256
    HF, HD = FM // 2, D // 2
    R3, R4, R2, RO = 0, Fd, 2 * Fd, 2 * Fd + D
    Q3 = 2 * Fd + 2 * D
    Q4, Q2, QO = Q3 + FM, Q3 + 2 * FM, Q3 + 2 * FM + D
    DUM = QO + D

    def cp(src, dst, k):
        return pltpu.make_async_copy(src, dst, sems.at[k])

    def cols(k):
        return (slice(None), pl.ds(k * D, D))

    copies = [
        [cp(wphi_hbm, wphi_v, 0), cp(gw_hbm, gw_v, 0)],
        [cp(wqkv_hbm.at[cols(1)], wqkv_v.at[cols(1)], 1)],
        [cp(x_hbm.at[pl.ds(0, T0)], x_v.at[pl.ds(0, T0)], 2)],
        [cp(w1_hbm, w1_v.at[pl.ds(0, D)], 3)],
        [cp(x_hbm.at[pl.ds(T0, T0)], x_v.at[pl.ds(T0, T0)], 4),
         cp(wqkv_hbm.at[cols(2)], wqkv_v.at[cols(2)], 4)],
    ]
    wsrc = {'3': (w3t_hbm.at[pl.ds(0, FM)], R3, FM), '4': (w4_hbm.at[pl.ds(0, FM)], R4, FM), '2': (w2_hbm, R2, D), 'o': (wo_hbm, RO, D)}

    def wcp(k, sem):
        return cp(wsrc[k][0], wf_v.at[pl.ds(wsrc[k][1], wsrc[k][2])], sem)

    XS = (2 + WPOS + ('+' in PAT1)) * T0 if EARLY else S
    g5 = [cp(x_hbm.at[pl.ds(2 * T0, XS - 2 * T0)], x_v.at[pl.ds(2 * T0, XS - 2 * T0)], 5)]
    g6 = []
    if EARLY:
        g5 += [wcp(k, 5) for k in EARLY]
        g6 += [cp(x_hbm.at[pl.ds(XS, S - XS)], x_v.at[pl.ds(XS, S - XS)], 6),
               cp(wqkv_hbm.at[cols(0)], wqkv_v.at[cols(0)], 6)]
    else:
        g5 += [cp(wqkv_hbm.at[cols(0)], wqkv_v.at[cols(0)], 5)]
    g6 += [wcp(k, 6) for k in '342o' if k not in EARLY]
    tl_ = pl.ds(FM, Fd - FM)
    g7 = [cp(w3t_hbm.at[tl_], wf_v.at[pl.ds(R3 + FM, Fd - FM)], 15),
          cp(w4_hbm.at[tl_], wf_v.at[pl.ds(R4 + FM, Fd - FM)], 15)]
    copies += [g5, g6, g7]
    bars = {int(b): cp(gw_hbm, bar_v.at[int(b)], 8 + int(b)) for b in BAR}
    for c in bars.values():
        c.start()
    for grp in copies:
        for c in grp:
            c.start()

    def wait(k):
        for c in copies[k]:
            c.wait()

    h_scr[:, 0:8, :] = jnp.zeros((4, 8, 128), F32)
    h_scr[:, S + 8:S + 16, :] = jnp.zeros((4, 8, 128), F32)

    def row_info(n):
        rr = lax.broadcasted_iota(jnp.int32, (D, n), 0)
        hg = rr // 128
        rr = rr % 128
        f = jnp.where(rr < 16, rr // 8, jnp.where(rr < 72, rr // 4 - 2, rr // 4 - 16))
        hl8 = jnp.where(rr < 16, rr % 8, jnp.where(rr < 72, rr % 4, 4 + rr % 4))
        return hg, f, hl8, lax.broadcasted_iota(jnp.int32, (D, n), 1)

    def fold(col0):
        lo = lax.broadcasted_iota(jnp.int32, (8, D), 0) < 4
        outs = []
        for hg in range(4):
            W = wqkv_v[:, col0 + hg * 128: col0 + (hg + 1) * 128]
            WT = lax.dot_general(p_s[hg * 128:(hg + 1) * 128, :], W, NT_DIMS,
                                 preferred_element_type=F32) * LOG2E
            ref = WT[0:8]
            rot = pltpu.roll(ref, 4, 0)
            outs.append(WT[8:16] - ref)
            outs.append((WT[16:72].reshape(7, 8, D) - jnp.where(lo, ref, rot)[None]).reshape(56, D))
            outs.append((WT[72:128].reshape(7, 8, D) - jnp.where(lo, rot, ref)[None]).reshape(56, D))
        return _pk(jnp.concatenate(outs, axis=0))

    def xt(t):
        return x_v[pl.ds(t[0], t[1]), :]

    def proj(w, t):
        return lax.dot_general(_up(w[...]), xt(t), NT_DIMS, preferred_element_type=F32)

    def sw_col(a, src, dst, H, n, wf_v=wf_v, z=None):
        if z is not None:
            src, dst = pl.multiple_of(src + z, 16), pl.multiple_of(dst + z, 16)
        l_, r_ = pl.ds(n * 128, 128), pl.ds(HD + n * 128, 128)
        lo_, hi_ = pl.ds(src, H), pl.ds(src + H, H)
        ta_, tb_ = pl.ds(dst, H), pl.ds(dst + H, H)
        return _wino_c(_nn, a, wf_v[lo_, l_], wf_v[hi_, l_], wf_v[hi_, r_],
                       wf_v[ta_, l_], wf_v[ta_, r_], wf_v[tb_, l_], wf_v[tb_, r_])

    def sw_nn(a, src, dst, H, ns, bank=wf_v, z=None):
        return sw_join([sw_col(a, src, dst, H, n, bank, z) for n in range(2)])

    def sw_join(cs_):
        top = jnp.concatenate([c[0] for c in cs_] + [c[1] for c in cs_], axis=1)
        bot = jnp.concatenate([c[2] for c in cs_] + [c[3] for c in cs_], axis=1)
        return top, bot

    def lhs7(a):
        top, bot = _split_rows(a)
        return [u.astype(BF16)
                for u in _wino_a(top[:, :HD], top[:, HD:], bot[:, :HD], bot[:, HD:])]

    def h_sw(t):
        xf = xt(t).astype(F32)
        m_, r_ = _ln_stats(xf)
        a7 = lhs7((xf - m_) * r_)
        for n in range(2):
            c11, c12, c21, c22 = sw_col(a7, 0, D, HD, n, w1_v)
            for g, y in ((n, _merge_rows(c11, c21)), (n + 2, _merge_rows(c12, c22))):
                h_scr[g, pl.ds(t[0] + 8, t[1]), :] = _gelu(y)
            yield None

    def phase1(step):
        wait(0)
        hg_, f_, hl8_, c = row_info(32)
        A = ((hg_ * 8 + hl8_) == c).astype(BF16)
        T1_ = lax.dot_general(A, wphi_v[...], NT_DIMS, preferred_element_type=F32)
        hg_, f_, hl8_, c = row_info(256)
        T2_ = jnp.where(f_ == (c % 16), T1_, 0.0).astype(BF16)
        r = lax.broadcasted_iota(jnp.int32, (256, 128), 0)
        c = lax.broadcasted_iota(jnp.int32, (256, 128), 1)
        Bm = ((r // 16) == (c % 16)).astype(BF16)
        P = jnp.dot(T2_, Bm, preferred_element_type=F32)
        hg_, f_, hl8_, c = row_info(128)
        p_s[...] = jnp.where(hl8_ == (c // 16), P, 0.0).astype(BF16)
        gw = gw_v[...].astype(F32)
        gwr = jnp.concatenate([gw[g:g + 1] for g in range(4)], axis=1)
        wkT[0:8, :] = _pk(jnp.broadcast_to(gwr, (16, D)))

        cs = []
        zs = [None] * 8
        kvs = [None] * 8

        def stats(t):
            return _ln_stats(xt(t).astype(F32))

        def h_stage(t, st):
            m, r = st
            if not cs:
                cs.append(jnp.sum(w1_v[0:D, :].astype(F32), axis=0, keepdims=True))
            y = jnp.dot(xt(t), w1_v[0:D, :], preferred_element_type=F32)
            h = _gelu((y - m * cs[0]) * r)
            for g in range(4):
                h_scr[g, pl.ds(t[0] + 8, t[1]), :] = h[:, g * 128:(g + 1) * 128]

        def k_soft(t, kT):
            n = t[1]
            gate = jax.nn.sigmoid(kT[0:8])
            for i in range(n // 128):
                g_s[t[0] // 128 + i] = gate[:, i * 128:(i + 1) * 128]
            ng_s[pl.ds(t[0], n), :] = jnp.concatenate([1.0 - gate] * 16, axis=0).T
            fks = []
            for g, pg in enumerate(_groups(kT[16:496])):
                ep, en, sp, sn = _exps(pg)
                fk = jnp.concatenate([(ep * _rcp(sp)[None]).reshape(64, n),
                                      (en * _rcp(sn)[None]).reshape(64, n)], axis=0)
                if not ZMX:
                    part = fk[:, 0:128]
                    for i in range(1, n // 128):
                        part = part + fk[:, i * 128:(i + 1) * 128]
                    zs[g] = part if zs[g] is None else zs[g] + part
                fks.append(fk.astype(BF16))
            return fks

        def v_split(vT):
            if ZMX:
                one = jnp.ones((16, vT.shape[1]), F32)
                return [jnp.concatenate([vT[g * 64:(g + 1) * 64, :], one], axis=0).astype(BF16)
                        for g in range(8)]
            return [vT[g * 64:(g + 1) * 64, :].astype(BF16) for g in range(8)]

        def kv_stage(fks, vT, gs=range(8)):
            for g in gs:
                part = lax.dot_general(vT[g], fks[g], NT_DIMS, preferred_element_type=F32)
                if ZMX:
                    part = part[0:72]
                kvs[g] = part if kvs[g] is None else kvs[g] + part

        off = pl.multiple_of(step * (-HD), 16)

        off8 = pl.multiple_of(step * (-64), 8)

        def pre(keys, part=0, parts=1, gates=None):
            tab = {'3': (R3, Q3, HF, True), '4': (R4, Q4, HF, False),
                   '2': (R2, Q2, HD, False), 'o': (RO, QO, HD, False)}
            tab['1'] = (0, D, HD, False)
            work = [(k, r0) for k in keys if k in SW + '34' for r0 in range(0, tab[k][2], RB)]
            n_ = -(-len(work) // parts)
            work = work[part * n_:(part + 1) * n_]
            for i_, (key, r0) in enumerate(work):
                src, dst, H, tr = tab[key]
                wf_ = w1_v if key == '1' else wf_v
                if gates is not None:
                    wf_[pl.ds(off + DUM, 8), 0:128] = gates[
                        i_ * len(gates) // len(work)].astype(BF16)
                if True:
                    lo_ = wf_[src + r0:src + r0 + RB, :].astype(F32)
                    hi_ = wf_[src + H + r0:src + H + r0 + RB, :].astype(F32)
                    if tr:
                        t1, t2, t3, t4 = _wino_b(lo_[:, :HD], hi_[:, :HD], lo_[:, HD:], hi_[:, HD:])
                    else:
                        t1, t2, t3, t4 = _wino_b(lo_[:, :HD], lo_[:, HD:], hi_[:, :HD], hi_[:, HD:])
                    wf_[pl.ds(off + dst + r0, RB), :] = jnp.concatenate(
                        [t1, t2], axis=1).astype(BF16)
                    wf_[pl.ds(off + dst + H + r0, RB), :] = jnp.concatenate(
                        [t3, t4], axis=1).astype(BF16)

        def v_stage(t):
            xb = xt(t)
            xf = xb.astype(F32)
            h = t[1] // 2
            tx = [u.astype(BF16) for u in
                  _wino_b(xf[:h, :HD], xf[h:, :HD], xf[:h, HD:], xf[h:, HD:])]
            q4 = D // 4
            av = (_up(wvT[0:q4, 0:HD]), _up(wvT[0:q4, HD:D]), _up(sv_s[3]),
                  _up(wvT[q4:2 * q4, HD:D]), _up(sv_s[0]), _up(sv_s[1]), _up(sv_s[2]))
            for c_ in _wino_gen(_nt, av, xb[:h, :HD], xb[:h, HD:], xb[h:, HD:], *tx):
                if c_ is None:
                    yield None
            c11, c12, c21, c22 = c_
            yield v_split(jnp.concatenate([jnp.concatenate([c11, c12], axis=1),
                                            jnp.concatenate([c21, c22], axis=1)], axis=0))

        ta, tb = (0, T0), (T0, T0)
        wait(1)
        wkT[8:248, :] = fold(D)
        wait(2)
        k0 = proj(wkT.at[0:248], ta)
        s0 = stats(ta)
        if S3:
            f0_ = k_soft(ta, k0)
        wait(3)
        h_stage(ta, s0)
        if P4:
            lo_ = w1_v[0:HD, :].astype(F32)
            hi_ = w1_v[HD:D, :].astype(F32)
            t1, t2, t3, t4 = _wino_b(lo_[:, :HD], lo_[:, HD:], hi_[:, :HD], hi_[:, HD:])
            w1_v[D:D + HD, :] = jnp.concatenate([t1, t2], axis=1).astype(BF16)
            w1_v[D + HD:2 * D, :] = jnp.concatenate([t3, t4], axis=1).astype(BF16)
        wait(4)
        r5 = {}
        for c in R5:
            if c == 'p' and not P4:
                pre('1')
            elif c == 'K':
                r5['k1'] = proj(wkT.at[0:248], tb)
            elif c == 'T':
                wvt = wqkv_v[:, 2 * D:3 * D].T
                wvT[...] = _pk(wvt)
                wf32 = wvt.astype(F32)
                _, _, s4, _, s1, s2, s3 = _wino_a(wf32[:HD, :HD], wf32[:HD, HD:],
                                                  wf32[HD:, :HD], wf32[HD:, HD:])
                for i, u in enumerate((s1, s2, s3, s4)):
                    sv_s[i] = _pk(u)
            elif c == 's':
                r5['f0'] = f0_ if S3 else k_soft(ta, k0)
            elif c == 't':
                r5['f1'] = k_soft(tb, r5['k1'])
            elif c in 'VW':
                r5['v' + str('VW'.index(c))] = v_split(proj(wvT, (ta, tb)['VW'.index(c)]))
            elif c in 'vw':
                r5['v' + str('vw'.index(c))] = list(v_stage((ta, tb)['vw'.index(c)]))[-1]
            elif c in 'AB':
                i = str('AB'.index(c))
                kv_stage(r5['f' + i], r5['v' + i])
            elif c == 'H':
                h_stage(tb, stats(tb))
            elif c == 'h':
                list(h_sw(tb))
        wait(5)
        tl = _tiles(T1, 2 * T0)
        s1_ = {}
        def step_gen(key, u, mk):
            if (key, u) not in s1_:
                s1_[key, u] = mk()
            r_ = next(s1_[key, u])
            if r_ is not None:
                s1_[key + 'r', u] = r_

        for it in range(-1, len(tl) + 1):
            if it in bars:
                bars[it].wait()
            if it == WPOS:
                wait(6)
            ea = [int(c) for c in GE] or [0] + [b for b in sorted(bars) if b < WPOS]
            la = [int(c) for c in GL] or [WPOS] + [b for b in sorted(bars) if b > WPOS]
            def do_pre(gates):
                if it in ea:
                    pre(EARLY, ea.index(it), len(ea), gates)
                if it in la:
                    pre([k for k in '342o' if k not in EARLY], la.index(it), len(la), gates)

            if not PACE:
                do_pre(None)
            if it == len(tl):
                wqT[...] = fold(0)
            for o in PAT1.split(','):
                u = it - (1 if o.endswith('-') else 0) + (1 if o.endswith('+') else 0)
                if not 0 <= u < len(tl):
                    continue
                t = tl[u]
                if o[0] == 'K':
                    if LINK and ('kv', u - LINK) in s1_:
                        wkT[pl.ds(off8 + 248, 8), 0:128] = pltpu.bitcast(s1_['kv', u - LINK], U32)
                    kT_ = lax.dot_general(_up(wkT[0:248, :]), xt(t), NT_DIMS,
                                          preferred_element_type=F32)
                    gk = [kT_[r * 8:(r + 1) * 8, n * 128:(n + 1) * 128]
                          for n in range(t[1] // 128) for r in range(62)]
                    TRACE.clear()
                    if PACE == '1':
                        do_pre(gk)
                    s1_['f', u] = k_soft(t, kT_)
                elif o[0] == 'v':
                    step_gen('v', u, lambda: v_stage(t))
                    if PACE > '1' and ('vr', u) in s1_:
                        gv = [a_[r * 8:(r + 1) * 8] for a_ in TRACE[:int(PACE) - 1]
                              for r in range(a_.shape[0] // 8)]
                        do_pre(gk + gv)
                elif o[0] == 'h':
                    if HMAP[u] != '-':
                        step_gen('h', u, lambda: h_sw(tl[int(HMAP[u])]))
                elif o[0] == 'a':
                    k_ = s1_.get(('a', u), 0)
                    s1_['a', u] = k_ + 2
                    kv_stage(s1_['f', u], s1_['vr', u], (k_, k_ + 1))
                    if k_ == 6:
                        acc_ = kvs[0][0:8]
                        for g_ in range(1, 8):
                            acc_ = acc_ + kvs[g_][0:8]
                        s1_['kv', u] = acc_
        for g in range(8):
            if ZMX:
                zb[g] = jnp.concatenate([kvs[g][64:72]] * 16, axis=0).T
            elif ZP == 'p2':
                z_s[g] = zs[g]
            else:
                zb[g] = jnp.broadcast_to(jnp.sum(zs[g], axis=1, keepdims=True), (128, 128))
        r = lax.broadcasted_iota(jnp.int32, (64, 128), 0)
        c = lax.broadcasted_iota(jnp.int32, (64, 128), 1)
        msk = (r // 16) == (c % 4)
        for g in range(8):
            kvT[g] = _pk(jnp.where(msk, kvs[g][0:64], 0.0))
        wait(7)

    def phase2(half):
        base = pl.multiple_of(half * (S // 2), S // 2)
        gbase = half * (S // 256)

        def w2_part(t, i):
            shifts = (-1, 1, -2, 2)
            n = t[1] // 2
            r0 = t[0] + i * n
            hsft = jnp.concatenate(
                [h_scr[g, pl.ds(r0 + 8 + shifts[g], n), :] for g in range(4)], axis=1)
            x1 = x_v[pl.ds(r0, n), :].astype(F32) + _merge_rows(*sw_nn(lhs7(hsft), R2, Q2, HD, 2))
            m, r = _ln_stats(x1)
            return x1, (x1 - m) * r

        def q_stage(t):
            n = t[1]
            qT = proj(wqT, t)
            gate = jnp.concatenate([g_s[gbase + t[2] // 128 + i] for i in range(n // 128)], axis=1)
            fqs = []
            for g, pg in enumerate(_groups(qT)):
                ep, en, sp, sn = _exps(pg)
                zt = jnp.concatenate([zb[g]] * (n // 128), axis=1)
                ap = _fold4(jnp.sum(ep * zt[0:64].reshape(8, 8, n), axis=0), jnp.add)
                an = _fold4(jnp.sum(en * zt[64:128].reshape(8, 8, n), axis=0), jnp.add)
                rd = gate * _rcp(ap * sn + an * sp + 1e-6 * (sp * sn))
                fq = jnp.concatenate([(ep * (sn * rd)[None]).reshape(64, n),
                                      (en * (sp * rd)[None]).reshape(64, n)], axis=0)
                fqs.append(fq)
            return fqs

        def num_stage(fqs):
            o = {g: _nn(_up(kvT[g]), fqs[g]) for g in (0, 4, 1, 5, 2, 6, 3, 7)}
            return jnp.concatenate([o[g] for g in range(8)], axis=0)

        def out_stage(t, oT, b, last):
            if 'o' in SW and not last:
                h = t[1] // 2
                a = [u.astype(BF16).T
                     for u in _wino_a(oT[:HD, :h], oT[HD:, :h], oT[:HD, h:], oT[HD:, h:])]
                res = jnp.concatenate(sw_nn(a, RO, QO, HD, 2), axis=0) + b
                idx = pl.ds(t[0], t[1])
                o_v[idx, :] = res.astype(BF16)
                cp(o_v.at[idx], out_hbm.at[idx], 7).start()
                return
            o = oT.astype(BF16).T
            sizes = [t[1]]
            if last:
                tail = [int(c) for c in CH.split(',')]
                sizes = [t[1] - sum(tail)] + tail
            a0 = 0
            for n in sizes:
                a = _nn(o[a0:a0 + n], wf_v[RO:RO + D, :])
                idx = pl.ds(t[0] + a0, n)
                o_v[idx, :] = (a + b[a0:a0 + n]).astype(BF16)
                cp(o_v.at[idx], out_hbm.at[idx], 7).start()
                a0 += n

        for g in range(8 if ZP == 'p2' else 0):
            zb[g] = jnp.broadcast_to(jnp.sum(z_s[g], axis=1, keepdims=True), (128, 128))
        ts = [(pl.multiple_of(base + a, 128), n, a) for a, n in _tiles(T2, 0)]
        st = {}

        def w4_gen(u):
            a11, a12, s4, a22, s1, s2, s3 = st['h3', u]
            ht, hb = _split_rows(st['hr', u])
            res = []
            for n in range(2):
                l_, r_ = pl.ds(n * 128, 128), pl.ds(HD + n * 128, 128)
                lo_, hx_ = pl.ds(R4, HF), pl.ds(R4 + HF, Fd - HF)
                ta_, tb_ = pl.ds(Q4, HF), pl.ds(Q4 + HF, HF)
                tail = pl.ds(R4 + FM, Fd - FM)
                p1 = _nn(a11, wf_v[lo_, l_])
                u2 = p1 + _nn(s2, wf_v[ta_, r_])
                c11 = p1 + _nn(jnp.concatenate([a12, ht], axis=1), wf_v[hx_, l_])
                yield
                u3 = u2 + _nn(s3, wf_v[tb_, l_])
                p5 = _nn(s1, wf_v[ta_, l_])
                c12 = u2 + p5 + _nn(jnp.concatenate([s4, ht], axis=1), wf_v[hx_, r_])
                yield
                c22 = u3 + p5 + _nn(hb, wf_v[tail, r_])
                c21 = u3 - _nn(a22, wf_v[tb_, r_]) + _nn(hb, wf_v[tail, l_])
                res.append((c11, c12, c21, c22))
                if n == 1:
                    st['y', u] = res
                yield

        def w3_gen(u):
            ln = jnp.concatenate([st.pop(('ln0', u)), st.pop(('ln1', u))], axis=0)
            a = lhs7(ln)
            outs = []
            for n in range(HF // 128):
                lo_ = pl.ds(R3 + n * 128, 128)
                hi_ = pl.ds(R3 + HF + n * 128, 128)
                ta_ = pl.ds(Q3 + n * 128, 128)
                tb_ = pl.ds(Q3 + HF + n * 128, 128)
                c = _wino_c(_nt, a, wf_v[lo_, 0:HD], wf_v[lo_, HD:D], wf_v[hi_, HD:D],
                            wf_v[ta_, 0:HD], wf_v[ta_, HD:D], wf_v[tb_, 0:HD], wf_v[tb_, HD:D])
                outs.append(_wino_a(*[_gelu(t) for t in c]))
                if n in (1, 3):
                    yield
            hr = _gelu(_nt(wf_v[R3 + FM:R3 + Fd, :], ln.astype(BF16))).astype(BF16)
            st['h3', u] = [jnp.concatenate([o[i] for o in outs], axis=1).astype(BF16)
                           for i in range(7)]
            st['hr', u] = hr.T
            yield

        def run(c, u):
            t = ts[u]
            if c == 'b':
                i = 0 if ('x10', u) not in st else 1
                st['x1%d' % i, u], st['ln%d' % i, u] = w2_part(t, i)
            elif c == 'q':
                i = 0 if ('q0', u) not in st else 1
                h = t[1] // 2
                st['q%d' % i, u] = q_stage((t[0] + i * h, h, t[2] + i * h))
            elif c in 'ce':
                if (c, u) not in st:
                    st[c, u] = w3_gen(u) if c == 'c' else w4_gen(u)
                next(st[c, u])
            elif c == 'N':
                st['oT', u] = num_stage([jnp.concatenate([a_, b_], axis=1).astype(BF16) for a_, b_ in
                                         zip(st.pop(('q0', u)), st.pop(('q1', u)))])
            elif c == 'O':
                y = _merge_rows(*sw_join(st.pop(('y', u))))
                b = jnp.concatenate([st.pop(('x10', u)), st.pop(('x11', u))], axis=0) + y
                b = b * jnp.concatenate([ng_s[pl.ds(t[0], t[1]), :]] * 4, axis=1)
                out_stage(t, st.pop(('oT', u)), b, u == len(ts) - 1)

        for c in PRO:
            run(c, 0)
        for u in range(len(ts)):
            for c in PAT2:
                v = u + (1 if c in 'bq' else 0)
                if v < len(ts):
                    run(c, v)

    def main(i, carry):
        if SKIP == '1':
            pl.when(i == 0)(lambda: [wait(k) for k in range(8)] and None)
        else:
            pl.when(i == 0)(lambda: phase1(i))
        if SKIP != '2':
            pl.when(i > 0)(lambda: phase2(i - 1))
        return carry

    lax.fori_loop(0, 3, main, 0)
    cp(o_v, out_hbm, 7).wait()


@jax.jit
def pallas_gated_mix__linear_kernel_hedgehog__mixer_s_mlp__prompt_kernel(
    A_x, A_wqkv, A_w_phi, A_wo, B_x, B_w1, B_w2, B_w3, B_w4, gate_w):
    B, S, D = A_x.shape
    Fd = B_w3.shape[1]
    x2 = A_x.reshape(S, D)
    wphi2 = A_w_phi.transpose(1, 2, 0).reshape(256, 32)
    gw2 = gate_w.reshape(4, 128)
    w3t = B_w3.T
    anyspec = pl.BlockSpec(memory_space=pl.ANY)
    out = pl.pallas_call(
        functools.partial(_kernel, S=S, D=D, Fd=Fd),
        in_specs=[anyspec] * 9,
        out_specs=anyspec,
        out_shape=jax.ShapeDtypeStruct((S, D), A_x.dtype),
        scratch_shapes=[
            pltpu.VMEM((S, D), BF16),
            pltpu.VMEM((D, 3 * D), BF16),
            pltpu.VMEM((256, 32), BF16),
            pltpu.VMEM((2 * D, D), BF16),
            pltpu.VMEM((4, D // 4, D // 2), U32),
            pltpu.VMEM((2 * Fd + 2 * (Fd // 256) * 256 + 4 * D + 16, D), BF16),
            pltpu.VMEM((4, 128), BF16),
            pltpu.VMEM((S, D), BF16),
            pltpu.VMEM((D, 128), BF16),
            pltpu.VMEM((256, D), U32),
            pltpu.VMEM((D // 2, D), U32),
            pltpu.VMEM((240, D), U32),
            pltpu.VMEM((4, S + 16, 128), F32),
            pltpu.VMEM((8, 32, 128), U32),
            pltpu.VMEM((8, 128, 128), F32),
            pltpu.VMEM((8, 128, 128), F32),
            pltpu.VMEM((S // 128, 8, 128), F32),
            pltpu.VMEM((S, 128), F32),
            pltpu.VMEM((8, 4, 128), BF16),
            pltpu.SemaphoreType.DMA((16,)),
        ],
        compiler_params=pltpu.CompilerParams(vmem_limit_bytes=100 * 1024 * 1024,
                                             disable_bounds_checks=True,
                                             disable_semaphore_checks=True),
    )(x2, A_wqkv, wphi2, A_wo, B_w1, B_w2, w3t, B_w4, gw2)
    return out.reshape(B, S, D)
```

```python
import functools

import jax
import jax.numpy as jnp
from jax import lax
import jax.experimental.pallas as pl
import jax.experimental.pallas.tpu as pltpu

F32 = jnp.float32
BF16 = jnp.bfloat16
U32 = jnp.uint32
TM = 256
IL = 16
RB = 8
GROUPS = (('x1', 'v'), ('x2', 'x3', '4'), ('x4', 'x5', 'x6', 'x7', 'q', '3', '2', 'o'))
SEQ1 = ('W4 T K1 V0 p1 h1 a0 v1 a1 W5 K2 v2 c40 h2 a2 K3 v3 c40 h3 a3 W6 Q '
        'K4 v4 c36 h4 a4 K5 v5 h5 c36 a5 K6 v6 c44 h6 a6 K7 c28 v7 h7 a7')
SEQ2 = ('b0 b0 q0 c0 c0 c0 e0 e0 e0 q1 q0 q1 e0 b1 N0 e0 e0 b1 O0 '
        'c1 c1 c1 e1 e1 q2 e1 q2 e1 b2 N1 e1 e1 b2 O1 '
        'c2 c2 c2 e2 e2 e2 q3 q3 e2 b3 N2 e2 e2 b3 O2 '
        'c3 c3 c3 e3 e3 e3 e3 N3 e3 e3 O3')
TAIL = (64, 48, 16)
NT_DIMS = (((1,), (1,)), ((), ()))
GC = 0.7978845608028654
LOG2E = 1.4426950408889634


def _gelu(x):
    return (0.5 * x) * (1.0 + jnp.tanh(x * (GC + (GC * 0.044715) * (x * x))))


def _rcp(x):
    return pl.reciprocal(x, approx=False, full_range=False)


def _ln_stats(xf):
    m = jnp.mean(xf, axis=-1, keepdims=True)
    v = jnp.maximum(jnp.mean(xf * xf, axis=-1, keepdims=True) - m * m, 0.0)
    return m, lax.rsqrt(v + 1e-5)


def _pk(x):
    return pltpu.bitcast(x.astype(BF16), U32)


def _up(x):
    return pltpu.bitcast(x, BF16)


def _nt(a, b):
    return lax.dot_general(a, b, NT_DIMS, preferred_element_type=F32)


def _nn(a, b):
    return jnp.dot(a, b, preferred_element_type=F32)


def _fold4(a, op):
    return op(a, pltpu.roll(a, 4, 0))


def _exps(p):
    p3 = p.reshape(8, 8, p.shape[1])
    mx = _fold4(jnp.max(p3, axis=0), jnp.maximum)
    mn = _fold4(jnp.min(p3, axis=0), jnp.minimum)
    ep = jnp.exp2(p3 - mx[None])
    en = jnp.exp2(mn[None] - p3)
    sp = _fold4(jnp.sum(ep, axis=0), jnp.add)
    sn = _fold4(jnp.sum(en, axis=0), jnp.add)
    return ep, en, sp, sn


def _groups(pT):
    lo = lax.broadcasted_iota(jnp.int32, (8, pT.shape[1]), 0) < 4
    for hg in range(4):
        blk = pT[hg * 120:(hg + 1) * 120]
        mid = blk[0:8]
        yield jnp.concatenate([jnp.where(lo, mid, 0.0), blk[8:64]], axis=0)
        yield jnp.concatenate([jnp.where(lo, 0.0, mid), blk[64:120]], axis=0)


def _wino_a(a11, a12, a21, a22):
    s1 = a21 + a22
    s2 = s1 - a11
    s3 = a11 - a21
    s4 = a12 - s2
    return a11, a12, s4, a22, s1, s2, s3


def _wino_b(b11, b12, b21, b22):
    t1 = b12 - b11
    t2 = b22 - t1
    t3 = b22 - b12
    t4 = t2 - b21
    return t1, t2, t3, t4


def _wino_c(mm, a, b11, b21, b22, t1, t2, t3, t4, trace=None):
    a11, a12, s4, a22, s1, s2, s3 = a
    p1 = mm(a11, b11)
    u2 = p1 + mm(s2, t2)
    c11 = p1 + mm(a12, b21)
    u3 = u2 + mm(s3, t3)
    p5 = mm(s1, t1)
    c12 = u2 + p5 + mm(s4, b22)
    c22 = u3 + p5
    c21 = u3 - mm(a22, t4)
    if trace is not None:
        trace += [u2, u3]
    return c11, c12, c21, c22


def _split_rows(a):
    m, n = a.shape
    a4 = a.reshape(m // (2 * IL), 2, IL, n)
    return a4[:, 0].reshape(m // 2, n), a4[:, 1].reshape(m // 2, n)


def _merge_rows(top, bot):
    h, n = top.shape
    return jnp.stack([top.reshape(h // IL, IL, n), bot.reshape(h // IL, IL, n)],
                     axis=1).reshape(2 * h, n)


def _kernel(x_hbm, wqkv_hbm, wphi_hbm, wo_hbm, w1_hbm, w2_hbm, w3t_hbm, w4_hbm, gw_hbm,
            out_hbm,
            x_v, wqkv_v, wphi_v, w1_v, sv_s, wf_v, gw_v, o_v,
            p_s, wkT, wvT, wqT, h_scr, kvT, zb, z_s, g_s, ng_s, sems,
            *, S, D, Fd):
    FM = (Fd // 256) * 256
    HF, HD = FM // 2, D // 2
    R3, R4, R2, RO = 0, Fd, 2 * Fd, 2 * Fd + D
    Q3 = 2 * Fd + 2 * D
    Q4, Q2, QO = Q3 + FM, Q3 + 2 * FM, Q3 + 2 * FM + D
    DUM = QO + D
    OSEM = 8

    def cp(src, dst, k):
        return pltpu.make_async_copy(src, dst, sems.at[k])

    def named(items, k):
        out = []
        xs = [int(i[1:]) for i in items if i[0] == 'x']
        for it in items:
            if it[0] == 'x':
                if int(it[1:]) == xs[0]:
                    r = pl.ds(xs[0] * TM, len(xs) * TM)
                    out.append(cp(x_hbm.at[r], x_v.at[r], k))
            elif it in 'qkv':
                c = (slice(None), pl.ds('qkv'.index(it) * D, D))
                out.append(cp(wqkv_hbm.at[c], wqkv_v.at[c], k))
            else:
                src, row, n = {'3': (w3t_hbm.at[pl.ds(0, FM)], R3, FM),
                               '4': (w4_hbm.at[pl.ds(0, FM)], R4, FM),
                               '2': (w2_hbm, R2, D), 'o': (wo_hbm, RO, D)}[it]
                out.append(cp(src, wf_v.at[pl.ds(row, n)], k))
        return out

    tail_rows = pl.ds(FM, Fd - FM)
    copies = [[cp(wphi_hbm, wphi_v, 0), cp(gw_hbm, gw_v, 0)], named(['k'], 1), named(['x0'], 2),
              [cp(w1_hbm, w1_v.at[pl.ds(0, D)], 3)]]
    copies += [named(g, 4 + i) for i, g in enumerate(GROUPS)]
    copies += [[cp(w3t_hbm.at[tail_rows], wf_v.at[pl.ds(R3 + FM, Fd - FM)], 7),
                cp(w4_hbm.at[tail_rows], wf_v.at[pl.ds(R4 + FM, Fd - FM)], 7)]]
    for grp in copies:
        for c in grp:
            c.start()

    def wait(k):
        for c in copies[k]:
            c.wait()

    h_scr[:, 0:8, :] = jnp.zeros((4, 8, 128), F32)
    h_scr[:, S + 8:S + 16, :] = jnp.zeros((4, 8, 128), F32)

    def row_info(n):
        rr = lax.broadcasted_iota(jnp.int32, (D, n), 0)
        hg = rr // 128
        rr = rr % 128
        f = jnp.where(rr < 16, rr // 8, jnp.where(rr < 72, rr // 4 - 2, rr // 4 - 16))
        hl8 = jnp.where(rr < 16, rr % 8, jnp.where(rr < 72, rr % 4, 4 + rr % 4))
        return hg, f, hl8, lax.broadcasted_iota(jnp.int32, (D, n), 1)

    def fold(col0):
        lo = lax.broadcasted_iota(jnp.int32, (8, D), 0) < 4
        outs = []
        for hg in range(4):
            W = wqkv_v[:, col0 + hg * 128: col0 + (hg + 1) * 128]
            WT = _nt(p_s[hg * 128:(hg + 1) * 128, :], W) * LOG2E
            ref = WT[0:8]
            rot = pltpu.roll(ref, 4, 0)
            outs.append(WT[8:16] - ref)
            outs.append((WT[16:72].reshape(7, 8, D) - jnp.where(lo, ref, rot)[None]).reshape(56, D))
            outs.append((WT[72:128].reshape(7, 8, D) - jnp.where(lo, rot, ref)[None]).reshape(56, D))
        return _pk(jnp.concatenate(outs, axis=0))

    def xr(r0, n):
        return x_v[pl.ds(r0, n), :]

    def sw_col(a, src, dst, H, n, bank):
        l_, r_ = pl.ds(n * 128, 128), pl.ds(HD + n * 128, 128)
        lo_, hi_ = pl.ds(src, H), pl.ds(src + H, H)
        ta_, tb_ = pl.ds(dst, H), pl.ds(dst + H, H)
        return _wino_c(_nn, a, bank[lo_, l_], bank[hi_, l_], bank[hi_, r_],
                       bank[ta_, l_], bank[ta_, r_], bank[tb_, l_], bank[tb_, r_])

    def sw_join(cs_):
        top = jnp.concatenate([c[0] for c in cs_] + [c[1] for c in cs_], axis=1)
        bot = jnp.concatenate([c[2] for c in cs_] + [c[3] for c in cs_], axis=1)
        return top, bot

    def lhs7(a):
        top, bot = _split_rows(a)
        return [u.astype(BF16)
                for u in _wino_a(top[:, :HD], top[:, HD:], bot[:, :HD], bot[:, HD:])]

    def phase1(step):
        wait(0)
        hg_, f_, hl8_, c = row_info(32)
        A = ((hg_ * 8 + hl8_) == c).astype(BF16)
        T1_ = _nt(A, wphi_v[...])
        hg_, f_, hl8_, c = row_info(256)
        T2_ = jnp.where(f_ == (c % 16), T1_, 0.0).astype(BF16)
        r = lax.broadcasted_iota(jnp.int32, (256, 128), 0)
        c = lax.broadcasted_iota(jnp.int32, (256, 128), 1)
        Bm = ((r // 16) == (c % 16)).astype(BF16)
        P = _nn(T2_, Bm)
        hg_, f_, hl8_, c = row_info(128)
        p_s[...] = jnp.where(hl8_ == (c // 16), P, 0.0).astype(BF16)
        gw = gw_v[...].astype(F32)
        gwr = jnp.concatenate([gw[g:g + 1] for g in range(4)], axis=1)
        wkT[0:8, :] = _pk(jnp.broadcast_to(gwr, (16, D)))

        zs = [None] * 8
        kvs = [None] * 8
        gates = []
        off = pl.multiple_of(step * (-HD), 16)

        def k_soft(j, kT):
            gate = jax.nn.sigmoid(kT[0:8])
            for i in range(2):
                g_s[2 * j + i] = gate[:, i * 128:(i + 1) * 128]
            ng_s[pl.ds(j * TM, TM), :] = jnp.concatenate([1.0 - gate] * 16, axis=0).T
            fks = []
            for g, pg in enumerate(_groups(kT[16:496])):
                ep, en, sp, sn = _exps(pg)
                fk = jnp.concatenate([(ep * _rcp(sp)[None]).reshape(64, TM),
                                      (en * _rcp(sn)[None]).reshape(64, TM)], axis=0)
                part = fk[:, 0:128] + fk[:, 128:256]
                zs[g] = part if zs[g] is None else zs[g] + part
                fks.append(fk.astype(BF16))
            return fks

        def v_split(vT):
            return [vT[g * 64:(g + 1) * 64, :].astype(BF16) for g in range(8)]

        def v_sw(j):
            xb = xr(j * TM, TM)
            xf = xb.astype(F32)
            h = TM // 2
            tx = [u.astype(BF16) for u in
                  _wino_b(xf[:h, :HD], xf[h:, :HD], xf[:h, HD:], xf[h:, HD:])]
            q4 = D // 4
            av = (_up(wvT[0:q4, 0:HD]), _up(wvT[0:q4, HD:D]), _up(sv_s[3]),
                  _up(wvT[q4:2 * q4, HD:D]), _up(sv_s[0]), _up(sv_s[1]), _up(sv_s[2]))
            tr = []
            c11, c12, c21, c22 = _wino_c(_nt, av, xb[:h, :HD], xb[:h, HD:], xb[h:, HD:], *tx, tr)
            gates.extend(a_[r * 8:(r + 1) * 8] for a_ in tr for r in range(HD // 8))
            return v_split(jnp.concatenate([jnp.concatenate([c11, c12], axis=1),
                                            jnp.concatenate([c21, c22], axis=1)], axis=0))

        def h_store(j, g, y):
            h_scr[g, pl.ds(j * TM + 8, TM), :] = _gelu(y)

        def h_sw(j):
            xf = xr(j * TM, TM).astype(F32)
            m_, r_ = _ln_stats(xf)
            a7 = lhs7((xf - m_) * r_)
            for n in range(2):
                c11, c12, c21, c22 = sw_col(a7, 0, D, HD, n, w1_v)
                h_store(j, n, _merge_rows(c11, c21))
                h_store(j, n + 2, _merge_rows(c12, c22))

        tab = {'3': (wf_v, R3, Q3, HF, True), '4': (wf_v, R4, Q4, HF, False),
               '2': (wf_v, R2, Q2, HD, False), 'o': (wf_v, RO, QO, HD, False),
               '1': (w1_v, 0, D, HD, False)}

        def piece(key, r0):
            bank, src, dst, H, tr = tab[key]
            lo_ = bank[src + r0:src + r0 + RB, :].astype(F32)
            hi_ = bank[src + H + r0:src + H + r0 + RB, :].astype(F32)
            if tr:
                t1, t2, t3, t4 = _wino_b(lo_[:, :HD], hi_[:, :HD], lo_[:, HD:], hi_[:, HD:])
            else:
                t1, t2, t3, t4 = _wino_b(lo_[:, :HD], lo_[:, HD:], hi_[:, :HD], hi_[:, HD:])
            bank[pl.ds(off + dst + r0, RB), :] = jnp.concatenate([t1, t2], axis=1).astype(BF16)
            bank[pl.ds(off + dst + H + r0, RB), :] = jnp.concatenate([t3, t4], axis=1).astype(BF16)

        work = [(k, r0) for k in '432o' for r0 in range(0, tab[k][3], RB)]

        wait(1)
        wkT[8:248, :] = fold(D)
        wait(2)
        st = {}
        k0 = _nt(_up(wkT[...]), xr(0, TM))
        m0, r0_ = _ln_stats(xr(0, TM).astype(F32))
        st['f', 0] = k_soft(0, k0)
        wait(3)
        cs = jnp.sum(w1_v[0:D, :].astype(F32), axis=0, keepdims=True)
        y = (_nn(xr(0, TM), w1_v[0:D, :]) - m0 * cs) * r0_
        for g in range(4):
            h_store(0, g, y[:, g * 128:(g + 1) * 128])
        for op in SEQ1.split():
            c, j = op[0], int(op[1:] or 0)
            if c == 'W':
                wait(j)
                gates.clear()
            elif c == 'p':
                for r0 in range(0, HD, RB):
                    piece('1', r0)
            elif c == 'K':
                kT = _nt(_up(wkT[...]), xr(j * TM, TM))
                gates.extend(kT[r * 8:(r + 1) * 8, n * 128:(n + 1) * 128]
                             for n in range(2) for r in range(62))
                st['f', j] = k_soft(j, kT)
            elif c == 'T':
                wvt = wqkv_v[:, 2 * D:3 * D].T
                wvT[...] = _pk(wvt)
                wf32 = wvt.astype(F32)
                _, _, s4, _, s1, s2, s3 = _wino_a(wf32[:HD, :HD], wf32[:HD, HD:],
                                                  wf32[HD:, :HD], wf32[HD:, HD:])
                for i, u in enumerate((s1, s2, s3, s4)):
                    sv_s[i] = _pk(u)
            elif c == 'V':
                st['v', j] = v_split(_nt(_up(wvT[...]), xr(j * TM, TM)))
            elif c == 'v':
                st['v', j] = v_sw(j)
            elif c == 'h':
                h_sw(j)
            elif c == 'a':
                fks, vT = st.pop(('f', j)), st.pop(('v', j))
                for g in range(8):
                    part = _nt(vT[g], fks[g])
                    kvs[g] = part if kvs[g] is None else kvs[g] + part
            elif c == 'Q':
                wqT[...] = fold(0)
            elif c == 'c':
                for i in range(j):
                    wf_v[pl.ds(off + DUM, 8), 0:128] = gates[i * len(gates) // j].astype(BF16)
                    piece(*work.pop(0))
                gates.clear()
        assert not work and not st
        r = lax.broadcasted_iota(jnp.int32, (64, 128), 0)
        c = lax.broadcasted_iota(jnp.int32, (64, 128), 1)
        msk = (r // 16) == (c % 4)
        for g in range(8):
            z_s[g] = zs[g]
            kvT[g] = _pk(jnp.where(msk, kvs[g], 0.0))
        wait(7)

    def phase2(half):
        base = pl.multiple_of(half * (S // 2), S // 2)
        gbase = half * (S // 256)
        HM = TM // 2
        last = S // (2 * TM) - 1

        def row(u, i=0):
            return pl.multiple_of(base + (u * TM + i * HM), HM)

        def w2_part(u, i):
            r0 = row(u, i)
            hsft = jnp.concatenate(
                [h_scr[g, pl.ds(r0 + 8 + sh, HM), :] for g, sh in enumerate((-1, 1, -2, 2))],
                axis=1)
            a7 = lhs7(hsft)
            hs = _merge_rows(*sw_join([sw_col(a7, R2, Q2, HD, n, wf_v) for n in range(2)]))
            x1 = xr(r0, HM).astype(F32) + hs
            m, r = _ln_stats(x1)
            return x1, (x1 - m) * r

        def q_part(u, i):
            qT = _nt(_up(wqT[...]), xr(row(u, i), HM))
            gate = g_s[gbase + 2 * u + i]
            fqs = []
            for g, pg in enumerate(_groups(qT)):
                ep, en, sp, sn = _exps(pg)
                z = zb[g]
                ap = _fold4(jnp.sum(ep * z[0:64].reshape(8, 8, HM), axis=0), jnp.add)
                an = _fold4(jnp.sum(en * z[64:128].reshape(8, 8, HM), axis=0), jnp.add)
                rd = gate * _rcp(ap * sn + an * sp + 1e-6 * (sp * sn))
                fqs.append(jnp.concatenate([(ep * (sn * rd)[None]).reshape(64, HM),
                                            (en * (sp * rd)[None]).reshape(64, HM)], axis=0))
            return fqs

        def emit(r0, n, val):
            idx = pl.ds(r0, n)
            o_v[idx, :] = val.astype(BF16)
            cp(o_v.at[idx], out_hbm.at[idx], OSEM).start()

        def out_stage(u, oT, b):
            a = [w.astype(BF16).T
                 for w in _wino_a(oT[:HD, :HM], oT[HD:, :HM], oT[:HD, HM:], oT[HD:, HM:])]
            if u == last:
                a0 = 0
                for n in TAIL:
                    ac = [w[a0:a0 + n] for w in a]
                    top, bot = sw_join([sw_col(ac, RO, QO, HD, k, wf_v) for k in range(2)])
                    emit(row(u) + a0, n, top + b[a0:a0 + n])
                    emit(row(u) + HM + a0, n, bot + b[HM + a0:HM + a0 + n])
                    a0 += n
            else:
                res = sw_join([sw_col(a, RO, QO, HD, n, wf_v) for n in range(2)])
                emit(row(u), TM, jnp.concatenate(res, axis=0) + b)

        st = {}

        def w3_gen(u):
            ln = jnp.concatenate([st.pop(('ln0', u)), st.pop(('ln1', u))], axis=0)
            a = lhs7(ln)
            outs = []
            for n in range(HF // 128):
                lo_ = pl.ds(R3 + n * 128, 128)
                hi_ = pl.ds(R3 + HF + n * 128, 128)
                ta_ = pl.ds(Q3 + n * 128, 128)
                tb_ = pl.ds(Q3 + HF + n * 128, 128)
                c = _wino_c(_nt, a, wf_v[lo_, 0:HD], wf_v[lo_, HD:D], wf_v[hi_, HD:D],
                            wf_v[ta_, 0:HD], wf_v[ta_, HD:D], wf_v[tb_, 0:HD], wf_v[tb_, HD:D])
                outs.append(_wino_a(*[_gelu(t) for t in c]))
                if n in (1, 3):
                    yield
            hr = _gelu(_nt(wf_v[R3 + FM:R3 + Fd, :], ln.astype(BF16))).astype(BF16)
            st['h3', u] = [jnp.concatenate([o[i] for o in outs], axis=1).astype(BF16)
                           for i in range(7)]
            st['hr', u] = hr.T
            yield

        def w4_gen(u):
            a11, a12, s4, a22, s1, s2, s3 = st['h3', u]
            ht, hb = _split_rows(st['hr', u])
            res = []
            for n in range(2):
                l_, r_ = pl.ds(n * 128, 128), pl.ds(HD + n * 128, 128)
                lo_, hx_ = pl.ds(R4, HF), pl.ds(R4 + HF, Fd - HF)
                ta_, tb_ = pl.ds(Q4, HF), pl.ds(Q4 + HF, HF)
                tail = pl.ds(R4 + FM, Fd - FM)
                p1 = _nn(a11, wf_v[lo_, l_])
                u2 = p1 + _nn(s2, wf_v[ta_, r_])
                c11 = p1 + _nn(jnp.concatenate([a12, ht], axis=1), wf_v[hx_, l_])
                yield
                u3 = u2 + _nn(s3, wf_v[tb_, l_])
                p5 = _nn(s1, wf_v[ta_, l_])
                c12 = u2 + p5 + _nn(jnp.concatenate([s4, ht], axis=1), wf_v[hx_, r_])
                yield
                c22 = u3 + p5 + _nn(hb, wf_v[tail, r_])
                c21 = u3 - _nn(a22, wf_v[tb_, r_]) + _nn(hb, wf_v[tail, l_])
                res.append((c11, c12, c21, c22))
                if n == 1:
                    st['y', u] = res
                yield

        for g in range(8):
            zb[g] = jnp.broadcast_to(jnp.sum(z_s[g], axis=1, keepdims=True), (128, 128))
        for op in SEQ2.split():
            c, u = op[0], int(op[1])
            if c == 'b':
                i = 0 if ('x10', u) not in st else 1
                st['x1%d' % i, u], st['ln%d' % i, u] = w2_part(u, i)
            elif c == 'q':
                i = 0 if ('q0', u) not in st else 1
                st['q%d' % i, u] = q_part(u, i)
            elif c in 'ce':
                if (c, u) not in st:
                    st[c, u] = w3_gen(u) if c == 'c' else w4_gen(u)
                next(st[c, u])
            elif c == 'N':
                fq = [jnp.concatenate([a_, b_], axis=1).astype(BF16)
                      for a_, b_ in zip(st.pop(('q0', u)), st.pop(('q1', u)))]
                o = {g: _nn(_up(kvT[g]), fq[g]) for g in (0, 4, 1, 5, 2, 6, 3, 7)}
                st['oT', u] = jnp.concatenate([o[g] for g in range(8)], axis=0)
            elif c == 'O':
                y = _merge_rows(*sw_join(st.pop(('y', u))))
                b = jnp.concatenate([st.pop(('x10', u)), st.pop(('x11', u))], axis=0) + y
                b = b * jnp.concatenate([ng_s[pl.ds(row(u), TM), :]] * 4, axis=1)
                out_stage(u, st.pop(('oT', u)), b)

    def main(i, carry):
        pl.when(i == 0)(lambda: phase1(i))
        pl.when(i > 0)(lambda: phase2(i - 1))
        return carry

    lax.fori_loop(0, 3, main, 0)
    cp(o_v, out_hbm, OSEM).wait()


@jax.jit
def pallas_gated_mix__linear_kernel_hedgehog__mixer_s_mlp__prompt_kernel(
    A_x: jax.Array,
    A_wqkv: jax.Array,
    A_w_phi: jax.Array,
    A_wo: jax.Array,
    B_x: jax.Array,
    B_w1: jax.Array,
    B_w2: jax.Array,
    B_w3: jax.Array,
    B_w4: jax.Array,
    gate_w: jax.Array,
):
    B, S, D = A_x.shape
    Fd = B_w3.shape[1]
    assert (B, S, D, Fd) == (1, 8 * TM, 512, 1376) and A_w_phi.shape == (32, 16, 16)
    FM = (Fd // 256) * 256
    x2 = A_x.reshape(S, D)
    wphi2 = A_w_phi.transpose(1, 2, 0).reshape(256, 32)
    gw2 = gate_w.reshape(4, 128)
    w3t = B_w3.T
    anyspec = pl.BlockSpec(memory_space=pl.ANY)
    out = pl.pallas_call(
        functools.partial(_kernel, S=S, D=D, Fd=Fd),
        in_specs=[anyspec] * 9,
        out_specs=anyspec,
        out_shape=jax.ShapeDtypeStruct((S, D), A_x.dtype),
        scratch_shapes=[
            pltpu.VMEM((S, D), BF16),
            pltpu.VMEM((D, 3 * D), BF16),
            pltpu.VMEM((256, 32), BF16),
            pltpu.VMEM((2 * D, D), BF16),
            pltpu.VMEM((4, D // 4, D // 2), U32),
            pltpu.VMEM((2 * Fd + 2 * FM + 4 * D + 16, D), BF16),
            pltpu.VMEM((4, 128), BF16),
            pltpu.VMEM((S, D), BF16),
            pltpu.VMEM((D, 128), BF16),
            pltpu.VMEM((248, D), U32),
            pltpu.VMEM((D // 2, D), U32),
            pltpu.VMEM((240, D), U32),
            pltpu.VMEM((4, S + 16, 128), F32),
            pltpu.VMEM((8, 32, 128), U32),
            pltpu.VMEM((8, 128, 128), F32),
            pltpu.VMEM((8, 128, 128), F32),
            pltpu.VMEM((S // 128, 8, 128), F32),
            pltpu.VMEM((S, 128), F32),
            pltpu.SemaphoreType.DMA((9,)),
        ],
        compiler_params=pltpu.CompilerParams(vmem_limit_bytes=100 * 1024 * 1024,
                                             disable_bounds_checks=True,
                                             disable_semaphore_checks=True),
    )(x2, A_wqkv, wphi2, A_wo, B_w1, B_w2, w3t, B_w4, gw2)
    return out.reshape(B, S, D)
```

```python
import functools

import jax
import jax.numpy as jnp
from jax import lax
import jax.experimental.pallas as pl
import jax.experimental.pallas.tpu as pltpu

F32 = jnp.float32
BF16 = jnp.bfloat16
U32 = jnp.uint32
TM = 256
IL = 16
RB = 8
GROUPS = (('x1', 'v'), ('x2', 'x3', 'x4', '4'), ('x5', 'x6', 'x7', 'q', '3', '2', 'o'))
SEQ1 = ('W4 K1 p1 T h1 V0 v1 a0 a1 W5 K2 v2 c32 a2 h2 K3 v3 h3 a3 c44 h4 W6 Q '
        'K4 v4 c28 a4 K5 v5 h5 a5 c40 K6 v6 c48 h6 a6 K7 c32 v7 h7 a7')
SEQ2 = ('b0 b0 q0 c0 c0 c0 e0 e0 e0 q1 q0 q1 e0 b1 N0 e0 e0 b1 O0 '
        'c1 c1 c1 e1 e1 e1 q2 q2 e1 b2 N1 e1 e1 b2 O1 '
        'c2 c2 c2 e2 e2 e2 q3 q3 e2 b3 N2 e2 e2 b3 O2 '
        'c3 c3 c3 e3 e3 e3 e3 N3 e3 e3 O3')
TAIL = (64, 48, 16)
NT_DIMS = (((1,), (1,)), ((), ()))
GC = 0.7978845608028654
LOG2E = 1.4426950408889634


def _gelu(x):
    return (0.5 * x) * (1.0 + jnp.tanh(x * (GC + (GC * 0.044715) * (x * x))))


def _rcp(x):
    return pl.reciprocal(x, approx=False, full_range=False)


def _ln_stats(xf):
    m = jnp.mean(xf, axis=-1, keepdims=True)
    v = jnp.maximum(jnp.mean(xf * xf, axis=-1, keepdims=True) - m * m, 0.0)
    return m, lax.rsqrt(v + 1e-5)


def _pk(x):
    return pltpu.bitcast(x.astype(BF16), U32)


def _up(x):
    return pltpu.bitcast(x, BF16)


def _nt(a, b):
    return lax.dot_general(a, b, NT_DIMS, preferred_element_type=F32)


def _nn(a, b):
    return jnp.dot(a, b, preferred_element_type=F32)


def _fold4(a, op):
    return op(a, pltpu.roll(a, 4, 0))


def _exps(p):
    p3 = p.reshape(8, 8, p.shape[1])
    mx = _fold4(jnp.max(p3, axis=0), jnp.maximum)
    mn = _fold4(jnp.min(p3, axis=0), jnp.minimum)
    ep = jnp.exp2(p3 - mx[None])
    en = jnp.exp2(mn[None] - p3)
    sp = _fold4(jnp.sum(ep, axis=0), jnp.add)
    sn = _fold4(jnp.sum(en, axis=0), jnp.add)
    return ep, en, sp, sn


def _groups(pT):
    lo = lax.broadcasted_iota(jnp.int32, (8, pT.shape[1]), 0) < 4
    for hg in range(4):
        blk = pT[hg * 120:(hg + 1) * 120]
        mid = blk[0:8]
        yield jnp.concatenate([jnp.where(lo, mid, 0.0), blk[8:64]], axis=0)
        yield jnp.concatenate([jnp.where(lo, 0.0, mid), blk[64:120]], axis=0)


def _wino_a(a11, a12, a21, a22):
    s1 = a21 + a22
    s2 = s1 - a11
    s3 = a11 - a21
    s4 = a12 - s2
    return a11, a12, s4, a22, s1, s2, s3


def _wino_b(b11, b12, b21, b22):
    t1 = b12 - b11
    t2 = b22 - t1
    t3 = b22 - b12
    t4 = t2 - b21
    return t1, t2, t3, t4


def _wino_c(mm, a, b11, b21, b22, t1, t2, t3, t4, trace=None):
    a11, a12, s4, a22, s1, s2, s3 = a
    p1 = mm(a11, b11)
    u2 = p1 + mm(s2, t2)
    c11 = p1 + mm(a12, b21)
    u3 = u2 + mm(s3, t3)
    p5 = mm(s1, t1)
    c12 = u2 + p5 + mm(s4, b22)
    c22 = u3 + p5
    c21 = u3 - mm(a22, t4)
    if trace is not None:
        trace += [u2, u3]
    return c11, c12, c21, c22


def _split_rows(a):
    m, n = a.shape
    a4 = a.reshape(m // (2 * IL), 2, IL, n)
    return a4[:, 0].reshape(m // 2, n), a4[:, 1].reshape(m // 2, n)


def _merge_rows(top, bot):
    h, n = top.shape
    return jnp.stack([top.reshape(h // IL, IL, n), bot.reshape(h // IL, IL, n)],
                     axis=1).reshape(2 * h, n)


def _kernel(x_hbm, wqkv_hbm, wphi_hbm, wo_hbm, w1_hbm, w2_hbm, w3t_hbm, w4_hbm, gw_hbm,
            out_hbm,
            x_v, wqkv_v, wphi_v, w1_v, sv_s, wf_v, gw_v, o_v,
            p_s, wkT, wvT, wqT, h_scr, kvT, zb, z_s, g_s, ng_s, sems,
            *, S, D, Fd):
    FM = (Fd // 256) * 256
    HF, HD = FM // 2, D // 2
    R3, R4, R2, RO = 0, Fd, 2 * Fd, 2 * Fd + D
    Q3 = 2 * Fd + 2 * D
    Q4, Q2, QO = Q3 + FM, Q3 + 2 * FM, Q3 + 2 * FM + D
    DUM = QO + D
    OSEM = 8

    def cp(src, dst, k):
        return pltpu.make_async_copy(src, dst, sems.at[k])

    def named(items, k):
        out = []
        xs = [int(i[1:]) for i in items if i[0] == 'x']
        for it in items:
            if it[0] == 'x':
                if int(it[1:]) == xs[0]:
                    r = pl.ds(xs[0] * TM, len(xs) * TM)
                    out.append(cp(x_hbm.at[r], x_v.at[r], k))
            elif it in 'qkv':
                c = (slice(None), pl.ds('qkv'.index(it) * D, D))
                out.append(cp(wqkv_hbm.at[c], wqkv_v.at[c], k))
            else:
                src, row, n = {'3': (w3t_hbm.at[pl.ds(0, FM)], R3, FM),
                               '4': (w4_hbm.at[pl.ds(0, FM)], R4, FM),
                               '2': (w2_hbm, R2, D), 'o': (wo_hbm, RO, D)}[it]
                out.append(cp(src, wf_v.at[pl.ds(row, n)], k))
        return out

    tail_rows = pl.ds(FM, Fd - FM)
    copies = [[cp(wphi_hbm, wphi_v, 0), cp(gw_hbm, gw_v, 0)], named(['k'], 1), named(['x0'], 2),
              [cp(w1_hbm, w1_v.at[pl.ds(0, D)], 3)]]
    copies += [named(g, 4 + i) for i, g in enumerate(GROUPS)]
    copies += [[cp(w3t_hbm.at[tail_rows], wf_v.at[pl.ds(R3 + FM, Fd - FM)], 7),
                cp(w4_hbm.at[tail_rows], wf_v.at[pl.ds(R4 + FM, Fd - FM)], 7)]]
    for grp in copies:
        for c in grp:
            c.start()

    def wait(k):
        for c in copies[k]:
            c.wait()

    h_scr[:, 0:8, :] = jnp.zeros((4, 8, 128), F32)
    h_scr[:, S + 8:S + 16, :] = jnp.zeros((4, 8, 128), F32)

    def row_info(n):
        rr = lax.broadcasted_iota(jnp.int32, (D, n), 0)
        hg = rr // 128
        rr = rr % 128
        f = jnp.where(rr < 16, rr // 8, jnp.where(rr < 72, rr // 4 - 2, rr // 4 - 16))
        hl8 = jnp.where(rr < 16, rr % 8, jnp.where(rr < 72, rr % 4, 4 + rr % 4))
        return hg, f, hl8, lax.broadcasted_iota(jnp.int32, (D, n), 1)

    def fold(col0):
        lo = lax.broadcasted_iota(jnp.int32, (8, D), 0) < 4
        outs = []
        for hg in range(4):
            W = wqkv_v[:, col0 + hg * 128: col0 + (hg + 1) * 128]
            WT = _nt(p_s[hg * 128:(hg + 1) * 128, :], W) * LOG2E
            ref = WT[0:8]
            rot = pltpu.roll(ref, 4, 0)
            outs.append(WT[8:16] - ref)
            outs.append((WT[16:72].reshape(7, 8, D) - jnp.where(lo, ref, rot)[None]).reshape(56, D))
            outs.append((WT[72:128].reshape(7, 8, D) - jnp.where(lo, rot, ref)[None]).reshape(56, D))
        return _pk(jnp.concatenate(outs, axis=0))

    def xr(r0, n):
        return x_v[pl.ds(r0, n), :]

    def sw_mm(a, src, dst, bank):
        lo_, hi_ = pl.ds(src, HD), pl.ds(src + HD, HD)
        ta_, tb_ = pl.ds(dst, HD), pl.ds(dst + HD, HD)
        return sw_join([_wino_c(_nn, a, bank[lo_, 0:HD], bank[hi_, 0:HD], bank[hi_, HD:D],
                                bank[ta_, 0:HD], bank[ta_, HD:D], bank[tb_, 0:HD],
                                bank[tb_, HD:D])])

    def sw_join(cs_):
        top = jnp.concatenate([c[0] for c in cs_] + [c[1] for c in cs_], axis=1)
        bot = jnp.concatenate([c[2] for c in cs_] + [c[3] for c in cs_], axis=1)
        return top, bot

    def lhs7(a):
        top, bot = _split_rows(a)
        return [u.astype(BF16)
                for u in _wino_a(top[:, :HD], top[:, HD:], bot[:, :HD], bot[:, HD:])]

    def phase1(step):
        wait(0)
        hg_, f_, hl8_, c = row_info(32)
        A = ((hg_ * 8 + hl8_) == c).astype(BF16)
        T1_ = _nt(A, wphi_v[...])
        hg_, f_, hl8_, c = row_info(256)
        T2_ = jnp.where(f_ == (c % 16), T1_, 0.0).astype(BF16)
        r = lax.broadcasted_iota(jnp.int32, (256, 128), 0)
        c = lax.broadcasted_iota(jnp.int32, (256, 128), 1)
        Bm = ((r // 16) == (c % 16)).astype(BF16)
        P = _nn(T2_, Bm)
        hg_, f_, hl8_, c = row_info(128)
        p_s[...] = jnp.where(hl8_ == (c // 16), P, 0.0).astype(BF16)
        gw = gw_v[...].astype(F32)
        gwr = jnp.concatenate([gw[g:g + 1] for g in range(4)], axis=1)
        wkT[0:8, :] = _pk(jnp.broadcast_to(gwr, (16, D)))

        zs = [None] * 8
        kvs = [None] * 8
        gates = []
        off = pl.multiple_of(step * (-HD), 16)

        def k_soft(j, kT):
            gate = jax.nn.sigmoid(kT[0:8])
            for i in range(2):
                g_s[2 * j + i] = gate[:, i * 128:(i + 1) * 128]
            ng_s[pl.ds(j * TM, TM), :] = jnp.concatenate([1.0 - gate] * 16, axis=0).T
            fks = []
            for g, pg in enumerate(_groups(kT[16:496])):
                ep, en, sp, sn = _exps(pg)
                fk = jnp.concatenate([(ep * _rcp(sp)[None]).reshape(64, TM),
                                      (en * _rcp(sn)[None]).reshape(64, TM)], axis=0)
                part = fk[:, 0:128] + fk[:, 128:256]
                zs[g] = part if zs[g] is None else zs[g] + part
                fks.append(fk.astype(BF16))
            return fks

        def v_split(vT):
            return [vT[g * 64:(g + 1) * 64, :].astype(BF16) for g in range(8)]

        def v_sw(j):
            xb = xr(j * TM, TM)
            xf = xb.astype(F32)
            h = TM // 2
            tx = [u.astype(BF16) for u in
                  _wino_b(xf[:h, :HD], xf[h:, :HD], xf[:h, HD:], xf[h:, HD:])]
            q4 = D // 4
            av = (_up(wvT[0:q4, 0:HD]), _up(wvT[0:q4, HD:D]), _up(sv_s[3]),
                  _up(wvT[q4:2 * q4, HD:D]), _up(sv_s[0]), _up(sv_s[1]), _up(sv_s[2]))
            tr = []
            c11, c12, c21, c22 = _wino_c(_nt, av, xb[:h, :HD], xb[:h, HD:], xb[h:, HD:], *tx, tr)
            gates.extend(a_[r * 8:(r + 1) * 8] for a_ in tr for r in range(HD // 8))
            return v_split(jnp.concatenate([jnp.concatenate([c11, c12], axis=1),
                                            jnp.concatenate([c21, c22], axis=1)], axis=0))

        def h_store(j, g, y):
            h_scr[g, pl.ds(j * TM + 8, TM), :] = _gelu(y)

        def h_sw(j):
            xf = xr(j * TM, TM).astype(F32)
            m_, r_ = _ln_stats(xf)
            a7 = lhs7((xf - m_) * r_)
            y = _merge_rows(*sw_mm(a7, 0, D, w1_v))
            for g in range(4):
                h_store(j, g, y[:, g * 128:(g + 1) * 128])

        tab = {'3': (wf_v, R3, Q3, HF, True), '4': (wf_v, R4, Q4, HF, False),
               '2': (wf_v, R2, Q2, HD, False), 'o': (wf_v, RO, QO, HD, False),
               '1': (w1_v, 0, D, HD, False)}

        def piece(key, r0):
            bank, src, dst, H, tr = tab[key]
            lo_ = bank[src + r0:src + r0 + RB, :].astype(F32)
            hi_ = bank[src + H + r0:src + H + r0 + RB, :].astype(F32)
            if tr:
                t1, t2, t3, t4 = _wino_b(lo_[:, :HD], hi_[:, :HD], lo_[:, HD:], hi_[:, HD:])
            else:
                t1, t2, t3, t4 = _wino_b(lo_[:, :HD], lo_[:, HD:], hi_[:, :HD], hi_[:, HD:])
            bank[pl.ds(off + dst + r0, RB), :] = jnp.concatenate([t1, t2], axis=1).astype(BF16)
            bank[pl.ds(off + dst + H + r0, RB), :] = jnp.concatenate([t3, t4], axis=1).astype(BF16)

        work = [(k, r0) for k in '432o' for r0 in range(0, tab[k][3], RB)]

        wait(1)
        wkT[8:248, :] = fold(D)
        wait(2)
        st = {}
        k0 = _nt(_up(wkT[...]), xr(0, TM))
        m0, r0_ = _ln_stats(xr(0, TM).astype(F32))
        st['f', 0] = k_soft(0, k0)
        wait(3)
        cs = jnp.sum(w1_v[0:D, :].astype(F32), axis=0, keepdims=True)
        y = (_nn(xr(0, TM), w1_v[0:D, :]) - m0 * cs) * r0_
        for g in range(4):
            h_store(0, g, y[:, g * 128:(g + 1) * 128])
        for op in SEQ1.split():
            c, j = op[0], int(op[1:] or 0)
            if c == 'W':
                wait(j)
                gates.clear()
            elif c == 'p':
                for r0 in range(0, HD, RB):
                    piece('1', r0)
            elif c == 'K':
                kT = _nt(_up(wkT[...]), xr(j * TM, TM))
                gates.extend(kT[r * 8:(r + 1) * 8, n * 128:(n + 1) * 128]
                             for n in range(2) for r in range(62))
                st['f', j] = k_soft(j, kT)
            elif c == 'T':
                wvt = wqkv_v[:, 2 * D:3 * D].T
                wvT[...] = _pk(wvt)
                wf32 = wvt.astype(F32)
                _, _, s4, _, s1, s2, s3 = _wino_a(wf32[:HD, :HD], wf32[:HD, HD:],
                                                  wf32[HD:, :HD], wf32[HD:, HD:])
                for i, u in enumerate((s1, s2, s3, s4)):
                    sv_s[i] = _pk(u)
            elif c == 'V':
                st['v', j] = v_split(_nt(_up(wvT[...]), xr(j * TM, TM)))
            elif c == 'v':
                st['v', j] = v_sw(j)
            elif c == 'h':
                h_sw(j)
            elif c == 'a':
                fks, vT = st.pop(('f', j)), st.pop(('v', j))
                for g in range(8):
                    part = _nt(vT[g], fks[g])
                    kvs[g] = part if kvs[g] is None else kvs[g] + part
            elif c == 'Q':
                wqT[...] = fold(0)
            elif c == 'c':
                for i in range(j):
                    wf_v[pl.ds(off + DUM, 8), 0:128] = gates[i * len(gates) // j].astype(BF16)
                    piece(*work.pop(0))
                gates.clear()
        assert not work and not st
        r = lax.broadcasted_iota(jnp.int32, (64, 128), 0)
        c = lax.broadcasted_iota(jnp.int32, (64, 128), 1)
        msk = (r // 16) == (c % 4)
        for g in range(8):
            z_s[g] = zs[g]
            kvT[g] = _pk(jnp.where(msk, kvs[g], 0.0))
        wait(7)

    def phase2(half):
        base = pl.multiple_of(half * (S // 2), S // 2)
        gbase = half * (S // 256)
        HM = TM // 2
        last = S // (2 * TM) - 1

        def row(u, i=0):
            return pl.multiple_of(base + (u * TM + i * HM), HM)

        def w2_part(u, i):
            r0 = row(u, i)
            hsft = jnp.concatenate(
                [h_scr[g, pl.ds(r0 + 8 + sh, HM), :] for g, sh in enumerate((-1, 1, -2, 2))],
                axis=1)
            a7 = lhs7(hsft)
            hs = _merge_rows(*sw_mm(a7, R2, Q2, wf_v))
            x1 = xr(r0, HM).astype(F32) + hs
            m, r = _ln_stats(x1)
            return x1, (x1 - m) * r

        def q_part(u, i):
            qT = _nt(_up(wqT[...]), xr(row(u, i), HM))
            gate = g_s[gbase + 2 * u + i]
            fqs = []
            for g, pg in enumerate(_groups(qT)):
                ep, en, sp, sn = _exps(pg)
                z = zb[g]
                ap = _fold4(jnp.sum(ep * z[0:64].reshape(8, 8, HM), axis=0), jnp.add)
                an = _fold4(jnp.sum(en * z[64:128].reshape(8, 8, HM), axis=0), jnp.add)
                rd = gate * _rcp(ap * sn + an * sp + 1e-6 * (sp * sn))
                fqs.append(jnp.concatenate([(ep * (sn * rd)[None]).reshape(64, HM),
                                            (en * (sp * rd)[None]).reshape(64, HM)], axis=0))
            return fqs

        def emit(r0, n, val):
            idx = pl.ds(r0, n)
            o_v[idx, :] = val.astype(BF16)
            cp(o_v.at[idx], out_hbm.at[idx], OSEM).start()

        def out_stage(u, oT, b):
            a = [w.astype(BF16).T
                 for w in _wino_a(oT[:HD, :HM], oT[HD:, :HM], oT[:HD, HM:], oT[HD:, HM:])]
            if u == last:
                a0 = 0
                for n in TAIL:
                    ac = [w[a0:a0 + n] for w in a]
                    top, bot = sw_mm(ac, RO, QO, wf_v)
                    emit(row(u) + a0, n, top + b[a0:a0 + n])
                    emit(row(u) + HM + a0, n, bot + b[HM + a0:HM + a0 + n])
                    a0 += n
            else:
                res = sw_mm(a, RO, QO, wf_v)
                emit(row(u), TM, jnp.concatenate(res, axis=0) + b)

        st = {}

        def w3_gen(u):
            ln = jnp.concatenate([st.pop(('ln0', u)), st.pop(('ln1', u))], axis=0)
            a = lhs7(ln)
            outs = []
            for n in range(HF // 128):
                lo_ = pl.ds(R3 + n * 128, 128)
                hi_ = pl.ds(R3 + HF + n * 128, 128)
                ta_ = pl.ds(Q3 + n * 128, 128)
                tb_ = pl.ds(Q3 + HF + n * 128, 128)
                c = _wino_c(_nt, a, wf_v[lo_, 0:HD], wf_v[lo_, HD:D], wf_v[hi_, HD:D],
                            wf_v[ta_, 0:HD], wf_v[ta_, HD:D], wf_v[tb_, 0:HD], wf_v[tb_, HD:D])
                outs.append(_wino_a(*[_gelu(t) for t in c]))
                if n in (1, 3):
                    yield
            hr = _gelu(_nt(wf_v[R3 + FM:R3 + Fd, :], ln.astype(BF16))).astype(BF16)
            st['h3', u] = [jnp.concatenate([o[i] for o in outs], axis=1).astype(BF16)
                           for i in range(7)]
            st['hr', u] = hr.T
            yield

        def w4_gen(u):
            a11, a12, s4, a22, s1, s2, s3 = st['h3', u]
            ht, hb = _split_rows(st['hr', u])
            res = []
            for n in range(2):
                l_, r_ = pl.ds(n * 128, 128), pl.ds(HD + n * 128, 128)
                lo_, hi_ = pl.ds(R4, HF), pl.ds(R4 + HF, HF)
                ta_, tb_ = pl.ds(Q4, HF), pl.ds(Q4 + HF, HF)
                tail = pl.ds(R4 + FM, Fd - FM)
                p1 = _nn(a11, wf_v[lo_, l_])
                u2 = p1 + _nn(s2, wf_v[ta_, r_])
                c11 = p1 + _nn(a12, wf_v[hi_, l_]) + _nn(ht, wf_v[tail, l_])
                yield
                u3 = u2 + _nn(s3, wf_v[tb_, l_])
                p5 = _nn(s1, wf_v[ta_, l_])
                c12 = u2 + p5 + _nn(s4, wf_v[hi_, r_]) + _nn(ht, wf_v[tail, r_])
                yield
                c22 = u3 + p5 + _nn(hb, wf_v[tail, r_])
                c21 = u3 - _nn(a22, wf_v[tb_, r_]) + _nn(hb, wf_v[tail, l_])
                res.append((c11, c12, c21, c22))
                if n == 1:
                    st['y', u] = res
                yield

        for g in range(8):
            zb[g] = jnp.broadcast_to(jnp.sum(z_s[g], axis=1, keepdims=True), (128, 128))
        for op in SEQ2.split():
            c, u = op[0], int(op[1])
            if c == 'b':
                i = 0 if ('x10', u) not in st else 1
                st['x1%d' % i, u], st['ln%d' % i, u] = w2_part(u, i)
            elif c == 'q':
                i = 0 if ('q0', u) not in st else 1
                st['q%d' % i, u] = q_part(u, i)
            elif c in 'ce':
                if (c, u) not in st:
                    st[c, u] = w3_gen(u) if c == 'c' else w4_gen(u)
                next(st[c, u])
            elif c == 'N':
                fq = [jnp.concatenate([a_, b_], axis=1).astype(BF16)
                      for a_, b_ in zip(st.pop(('q0', u)), st.pop(('q1', u)))]
                o = {g: _nn(_up(kvT[g]), fq[g]) for g in (0, 4, 1, 5, 2, 6, 3, 7)}
                st['oT', u] = jnp.concatenate([o[g] for g in range(8)], axis=0)
            elif c == 'O':
                y = _merge_rows(*sw_join(st.pop(('y', u))))
                b = jnp.concatenate([st.pop(('x10', u)), st.pop(('x11', u))], axis=0) + y
                b = b * jnp.concatenate([ng_s[pl.ds(row(u), TM), :]] * 4, axis=1)
                out_stage(u, st.pop(('oT', u)), b)

    def main(i, carry):
        pl.when(i == 0)(lambda: phase1(i))
        pl.when(i > 0)(lambda: phase2(i - 1))
        return carry

    lax.fori_loop(0, 3, main, 0)
    cp(o_v, out_hbm, OSEM).wait()


@jax.jit
def pallas_gated_mix__linear_kernel_hedgehog__mixer_s_mlp__prompt_kernel(
    A_x: jax.Array,
    A_wqkv: jax.Array,
    A_w_phi: jax.Array,
    A_wo: jax.Array,
    B_x: jax.Array,
    B_w1: jax.Array,
    B_w2: jax.Array,
    B_w3: jax.Array,
    B_w4: jax.Array,
    gate_w: jax.Array,
):
    B, S, D = A_x.shape
    Fd = B_w3.shape[1]
    assert (B, S, D, Fd) == (1, 8 * TM, 512, 1376) and A_w_phi.shape == (32, 16, 16)
    FM = (Fd // 256) * 256
    x2 = A_x.reshape(S, D)
    wphi2 = A_w_phi.transpose(1, 2, 0).reshape(256, 32)
    gw2 = gate_w.reshape(4, 128)
    w3t = B_w3.T
    anyspec = pl.BlockSpec(memory_space=pl.ANY)
    out = pl.pallas_call(
        functools.partial(_kernel, S=S, D=D, Fd=Fd),
        in_specs=[anyspec] * 9,
        out_specs=anyspec,
        out_shape=jax.ShapeDtypeStruct((S, D), A_x.dtype),
        scratch_shapes=[
            pltpu.VMEM((S, D), BF16),
            pltpu.VMEM((D, 3 * D), BF16),
            pltpu.VMEM((256, 32), BF16),
            pltpu.VMEM((2 * D, D), BF16),
            pltpu.VMEM((4, D // 4, D // 2), U32),
            pltpu.VMEM((2 * Fd + 2 * FM + 4 * D + 16, D), BF16),
            pltpu.VMEM((4, 128), BF16),
            pltpu.VMEM((S, D), BF16),
            pltpu.VMEM((D, 128), BF16),
            pltpu.VMEM((248, D), U32),
            pltpu.VMEM((D // 2, D), U32),
            pltpu.VMEM((240, D), U32),
            pltpu.VMEM((4, S + 16, 128), F32),
            pltpu.VMEM((8, 32, 128), U32),
            pltpu.VMEM((8, 128, 128), F32),
            pltpu.VMEM((8, 128, 128), F32),
            pltpu.VMEM((S // 128, 8, 128), F32),
            pltpu.VMEM((S, 128), F32),
            pltpu.SemaphoreType.DMA((9,)),
        ],
        compiler_params=pltpu.CompilerParams(vmem_limit_bytes=100 * 1024 * 1024,
                                             disable_bounds_checks=True,
                                             disable_semaphore_checks=True),
    )(x2, A_wqkv, wphi2, A_wo, B_w1, B_w2, w3t, B_w4, gw2)
    return out.reshape(B, S, D)
```

```python
import functools

import jax
import jax.numpy as jnp
from jax import lax
import jax.experimental.pallas as pl
import jax.experimental.pallas.tpu as pltpu

F32 = jnp.float32
BF16 = jnp.bfloat16
U32 = jnp.uint32
TM = 256
IL = 16
RB = 8
GROUPS = (('x1', 'v'), ('x2', 'x3', 'x4', '4'), ('x5', 'x6', 'x7', 'q', '3', '2', 'o'))
SEQ1 = ('W4 K1 p1 T h1 V0 v1 a0 a1 W5 K2 v2 c32 a2 h2 K3 v3 h3 a3 c44 h4 W6 Q '
        'K4 v4 c28 a4 K5 v5 h5 a5 c40 K6 v6 c48 h6 a6 K7 c32 v7 h7 a7')
SEQ2 = ('b0 b0 q0 b1 c0 c0 c0 e0 e0 b1 e0 c1 q0 e0 N0 e0 c1 b2 c1 e0 b2 O0 '
        'e1 q1 c2 c2 q1 e1 e1 e1 N1 e1 b3 e1 O1 b3 c2 e2 q2 q2 e2 e2 c3 e2 N2 e2 c3 e2 c3 O2 '
        'q3 e3 e3 q3 e3 N3 e3 e3 e3 O3')
TAIL = (64, 48, 16)
NT_DIMS = (((1,), (1,)), ((), ()))
GC = 0.7978845608028654
LOG2E = 1.4426950408889634


def _gelu(x):
    return (0.5 * x) * (1.0 + jnp.tanh(x * (GC + (GC * 0.044715) * (x * x))))


def _rcp(x):
    return pl.reciprocal(x, approx=False, full_range=False)


def _ln_stats(xf):
    m = jnp.mean(xf, axis=-1, keepdims=True)
    v = jnp.maximum(jnp.mean(xf * xf, axis=-1, keepdims=True) - m * m, 0.0)
    return m, lax.rsqrt(v + 1e-5)


def _pk(x):
    return pltpu.bitcast(x.astype(BF16), U32)


def _up(x):
    return pltpu.bitcast(x, BF16)


def _nt(a, b):
    return lax.dot_general(a, b, NT_DIMS, preferred_element_type=F32)


def _nn(a, b):
    return jnp.dot(a, b, preferred_element_type=F32)


def _fold4(a, op):
    return op(a, pltpu.roll(a, 4, 0))


def _exps(p):
    p3 = p.reshape(8, 8, p.shape[1])
    mx = _fold4(jnp.max(p3, axis=0), jnp.maximum)
    mn = _fold4(jnp.min(p3, axis=0), jnp.minimum)
    ep = jnp.exp2(p3 - mx[None])
    en = jnp.exp2(mn[None] - p3)
    sp = _fold4(jnp.sum(ep, axis=0), jnp.add)
    sn = _fold4(jnp.sum(en, axis=0), jnp.add)
    return ep, en, sp, sn


def _groups(pT):
    lo = lax.broadcasted_iota(jnp.int32, (8, pT.shape[1]), 0) < 4
    for hg in range(4):
        blk = pT[hg * 120:(hg + 1) * 120]
        mid = blk[0:8]
        yield jnp.concatenate([jnp.where(lo, mid, 0.0), blk[8:64]], axis=0)
        yield jnp.concatenate([jnp.where(lo, 0.0, mid), blk[64:120]], axis=0)


def _wino_a(a11, a12, a21, a22):
    s1 = a21 + a22
    s2 = s1 - a11
    s3 = a11 - a21
    s4 = a12 - s2
    return a11, a12, s4, a22, s1, s2, s3


def _wino_b(b11, b12, b21, b22):
    t1 = b12 - b11
    t2 = b22 - t1
    t3 = b22 - b12
    t4 = t2 - b21
    return t1, t2, t3, t4


def _wino_c(mm, a, b11, b21, b22, t1, t2, t3, t4, trace=None):
    a11, a12, s4, a22, s1, s2, s3 = a
    p1 = mm(a11, b11)
    u2 = p1 + mm(s2, t2)
    c11 = p1 + mm(a12, b21)
    u3 = u2 + mm(s3, t3)
    p5 = mm(s1, t1)
    c12 = u2 + p5 + mm(s4, b22)
    c22 = u3 + p5
    c21 = u3 - mm(a22, t4)
    if trace is not None:
        trace += [u2, u3]
    return c11, c12, c21, c22


def _split_rows(a):
    m, n = a.shape
    a4 = a.reshape(m // (2 * IL), 2, IL, n)
    return a4[:, 0].reshape(m // 2, n), a4[:, 1].reshape(m // 2, n)


def _merge_rows(top, bot):
    h, n = top.shape
    return jnp.stack([top.reshape(h // IL, IL, n), bot.reshape(h // IL, IL, n)],
                     axis=1).reshape(2 * h, n)


def _kernel(x_hbm, wqkv_hbm, wphi_hbm, wo_hbm, w1_hbm, w2_hbm, w3t_hbm, w4_hbm, gw_hbm,
            out_hbm,
            x_v, wqkv_v, wphi_v, w1_v, sv_s, wf_v, gw_v, o_v,
            p_s, wkT, wvT, wqT, h_scr, kvT, zb, z_s, g_s, ng_s, sems,
            *, S, D, Fd):
    FM = (Fd // 256) * 256
    HF, HD = FM // 2, D // 2
    R3, R4, R2, RO = 0, Fd, 2 * Fd, 2 * Fd + D
    Q3 = 2 * Fd + 2 * D
    Q4, Q2, QO = Q3 + FM, Q3 + 2 * FM, Q3 + 2 * FM + D
    DUM = QO + D
    OSEM = 8

    def cp(src, dst, k):
        return pltpu.make_async_copy(src, dst, sems.at[k])

    def named(items, k):
        out = []
        xs = [int(i[1:]) for i in items if i[0] == 'x']
        for it in items:
            if it[0] == 'x':
                if int(it[1:]) == xs[0]:
                    r = pl.ds(xs[0] * TM, len(xs) * TM)
                    out.append(cp(x_hbm.at[r], x_v.at[r], k))
            elif it in 'qkv':
                c = (slice(None), pl.ds('qkv'.index(it) * D, D))
                out.append(cp(wqkv_hbm.at[c], wqkv_v.at[c], k))
            else:
                src, row, n = {'3': (w3t_hbm.at[pl.ds(0, FM)], R3, FM),
                               '4': (w4_hbm.at[pl.ds(0, FM)], R4, FM),
                               '2': (w2_hbm, R2, D), 'o': (wo_hbm, RO, D)}[it]
                out.append(cp(src, wf_v.at[pl.ds(row, n)], k))
        return out

    tail_rows = pl.ds(FM, Fd - FM)
    copies = [[cp(wphi_hbm, wphi_v, 0), cp(gw_hbm, gw_v, 0)], named(['k'], 1), named(['x0'], 2),
              [cp(w1_hbm, w1_v.at[pl.ds(0, D)], 3)]]
    copies += [named(g, 4 + i) for i, g in enumerate(GROUPS)]
    copies += [[cp(w3t_hbm.at[tail_rows], wf_v.at[pl.ds(R3 + FM, Fd - FM)], 7),
                cp(w4_hbm.at[tail_rows], wf_v.at[pl.ds(R4 + FM, Fd - FM)], 7)]]
    for grp in copies:
        for c in grp:
            c.start()

    def wait(k):
        for c in copies[k]:
            c.wait()

    h_scr[:, 0:8, :] = jnp.zeros((4, 8, 128), F32)
    h_scr[:, S + 8:S + 16, :] = jnp.zeros((4, 8, 128), F32)

    def row_info(n):
        rr = lax.broadcasted_iota(jnp.int32, (D, n), 0)
        hg = rr // 128
        rr = rr % 128
        f = jnp.where(rr < 16, rr // 8, jnp.where(rr < 72, rr // 4 - 2, rr // 4 - 16))
        hl8 = jnp.where(rr < 16, rr % 8, jnp.where(rr < 72, rr % 4, 4 + rr % 4))
        return hg, f, hl8, lax.broadcasted_iota(jnp.int32, (D, n), 1)

    def fold(col0):
        lo = lax.broadcasted_iota(jnp.int32, (8, D), 0) < 4
        outs = []
        for hg in range(4):
            W = wqkv_v[:, col0 + hg * 128: col0 + (hg + 1) * 128]
            WT = _nt(p_s[hg * 128:(hg + 1) * 128, :], W) * LOG2E
            ref = WT[0:8]
            rot = pltpu.roll(ref, 4, 0)
            outs.append(WT[8:16] - ref)
            outs.append((WT[16:72].reshape(7, 8, D) - jnp.where(lo, ref, rot)[None]).reshape(56, D))
            outs.append((WT[72:128].reshape(7, 8, D) - jnp.where(lo, rot, ref)[None]).reshape(56, D))
        return _pk(jnp.concatenate(outs, axis=0))

    def xr(r0, n):
        return x_v[pl.ds(r0, n), :]

    def sw_mm(a, src, dst, bank):
        lo_, hi_ = pl.ds(src, HD), pl.ds(src + HD, HD)
        ta_, tb_ = pl.ds(dst, HD), pl.ds(dst + HD, HD)
        return sw_join([_wino_c(_nn, a, bank[lo_, 0:HD], bank[hi_, 0:HD], bank[hi_, HD:D],
                                bank[ta_, 0:HD], bank[ta_, HD:D], bank[tb_, 0:HD],
                                bank[tb_, HD:D])])

    def sw_join(cs_):
        top = jnp.concatenate([c[0] for c in cs_] + [c[1] for c in cs_], axis=1)
        bot = jnp.concatenate([c[2] for c in cs_] + [c[3] for c in cs_], axis=1)
        return top, bot

    def lhs7(a):
        top, bot = _split_rows(a)
        return [u.astype(BF16)
                for u in _wino_a(top[:, :HD], top[:, HD:], bot[:, :HD], bot[:, HD:])]

    def phase1(step):
        wait(0)
        hg_, f_, hl8_, c = row_info(32)
        A = ((hg_ * 8 + hl8_) == c).astype(BF16)
        T1_ = _nt(A, wphi_v[...])
        hg_, f_, hl8_, c = row_info(256)
        T2_ = jnp.where(f_ == (c % 16), T1_, 0.0).astype(BF16)
        r = lax.broadcasted_iota(jnp.int32, (256, 128), 0)
        c = lax.broadcasted_iota(jnp.int32, (256, 128), 1)
        Bm = ((r // 16) == (c % 16)).astype(BF16)
        P = _nn(T2_, Bm)
        hg_, f_, hl8_, c = row_info(128)
        p_s[...] = jnp.where(hl8_ == (c // 16), P, 0.0).astype(BF16)
        gw = gw_v[...].astype(F32)
        gwr = jnp.concatenate([gw[g:g + 1] for g in range(4)], axis=1)
        wkT[0:8, :] = _pk(jnp.broadcast_to(gwr, (16, D)))

        zs = [None] * 8
        kvs = [None] * 8
        gates = []
        off = pl.multiple_of(step * (-HD), 16)

        def k_soft(j, kT):
            gate = jax.nn.sigmoid(kT[0:8])
            for i in range(2):
                g_s[2 * j + i] = gate[:, i * 128:(i + 1) * 128]
            ng_s[pl.ds(j * TM, TM), :] = jnp.concatenate([1.0 - gate] * 16, axis=0).T
            fks = []
            for g, pg in enumerate(_groups(kT[16:496])):
                ep, en, sp, sn = _exps(pg)
                fk = jnp.concatenate([(ep * _rcp(sp)[None]).reshape(64, TM),
                                      (en * _rcp(sn)[None]).reshape(64, TM)], axis=0)
                part = fk[:, 0:128] + fk[:, 128:256]
                zs[g] = part if zs[g] is None else zs[g] + part
                fks.append(fk.astype(BF16))
            return fks

        def v_split(vT):
            return [vT[g * 64:(g + 1) * 64, :].astype(BF16) for g in range(8)]

        def v_sw(j):
            xb = xr(j * TM, TM)
            xf = xb.astype(F32)
            h = TM // 2
            tx = [u.astype(BF16) for u in
                  _wino_b(xf[:h, :HD], xf[h:, :HD], xf[:h, HD:], xf[h:, HD:])]
            q4 = D // 4
            av = (_up(wvT[0:q4, 0:HD]), _up(wvT[0:q4, HD:D]), _up(sv_s[3]),
                  _up(wvT[q4:2 * q4, HD:D]), _up(sv_s[0]), _up(sv_s[1]), _up(sv_s[2]))
            tr = []
            c11, c12, c21, c22 = _wino_c(_nt, av, xb[:h, :HD], xb[:h, HD:], xb[h:, HD:], *tx, tr)
            gates.extend(a_[r * 8:(r + 1) * 8] for a_ in tr for r in range(HD // 8))
            return v_split(jnp.concatenate([jnp.concatenate([c11, c12], axis=1),
                                            jnp.concatenate([c21, c22], axis=1)], axis=0))

        def h_store(j, g, y):
            h_scr[g, pl.ds(j * TM + 8, TM), :] = _gelu(y)

        def h_sw(j):
            xf = xr(j * TM, TM).astype(F32)
            m_, r_ = _ln_stats(xf)
            a7 = lhs7((xf - m_) * r_)
            y = _merge_rows(*sw_mm(a7, 0, D, w1_v))
            for g in range(4):
                h_store(j, g, y[:, g * 128:(g + 1) * 128])

        tab = {'3': (wf_v, R3, Q3, HF, True), '4': (wf_v, R4, Q4, HF, False),
               '2': (wf_v, R2, Q2, HD, False), 'o': (wf_v, RO, QO, HD, False),
               '1': (w1_v, 0, D, HD, False)}

        def piece(key, r0):
            bank, src, dst, H, tr = tab[key]
            lo_ = bank[src + r0:src + r0 + RB, :].astype(F32)
            hi_ = bank[src + H + r0:src + H + r0 + RB, :].astype(F32)
            if tr:
                t1, t2, t3, t4 = _wino_b(lo_[:, :HD], hi_[:, :HD], lo_[:, HD:], hi_[:, HD:])
            else:
                t1, t2, t3, t4 = _wino_b(lo_[:, :HD], lo_[:, HD:], hi_[:, :HD], hi_[:, HD:])
            bank[pl.ds(off + dst + r0, RB), :] = jnp.concatenate([t1, t2], axis=1).astype(BF16)
            bank[pl.ds(off + dst + H + r0, RB), :] = jnp.concatenate([t3, t4], axis=1).astype(BF16)

        work = [(k, r0) for k in '432o' for r0 in range(0, tab[k][3], RB)]

        wait(1)
        wkT[8:248, :] = fold(D)
        wait(2)
        st = {}
        k0 = _nt(_up(wkT[...]), xr(0, TM))
        m0, r0_ = _ln_stats(xr(0, TM).astype(F32))
        st['f', 0] = k_soft(0, k0)
        wait(3)
        cs = jnp.sum(w1_v[0:D, :].astype(F32), axis=0, keepdims=True)
        y = (_nn(xr(0, TM), w1_v[0:D, :]) - m0 * cs) * r0_
        for g in range(4):
            h_store(0, g, y[:, g * 128:(g + 1) * 128])
        for op in SEQ1.split():
            c, j = op[0], int(op[1:] or 0)
            if c == 'W':
                wait(j)
                gates.clear()
            elif c == 'p':
                for r0 in range(0, HD, RB):
                    piece('1', r0)
            elif c == 'K':
                kT = _nt(_up(wkT[...]), xr(j * TM, TM))
                gates.extend(kT[r * 8:(r + 1) * 8, n * 128:(n + 1) * 128]
                             for n in range(2) for r in range(62))
                st['f', j] = k_soft(j, kT)
            elif c == 'T':
                wvt = wqkv_v[:, 2 * D:3 * D].T
                wvT[...] = _pk(wvt)
                wf32 = wvt.astype(F32)
                _, _, s4, _, s1, s2, s3 = _wino_a(wf32[:HD, :HD], wf32[:HD, HD:],
                                                  wf32[HD:, :HD], wf32[HD:, HD:])
                for i, u in enumerate((s1, s2, s3, s4)):
                    sv_s[i] = _pk(u)
            elif c == 'V':
                st['v', j] = v_split(_nt(_up(wvT[...]), xr(j * TM, TM)))
            elif c == 'v':
                st['v', j] = v_sw(j)
            elif c == 'h':
                h_sw(j)
            elif c == 'a':
                fks, vT = st.pop(('f', j)), st.pop(('v', j))
                for g in range(8):
                    part = _nt(vT[g], fks[g])
                    kvs[g] = part if kvs[g] is None else kvs[g] + part
            elif c == 'Q':
                wqT[...] = fold(0)
            elif c == 'c':
                for i in range(j):
                    wf_v[pl.ds(off + DUM, 8), 0:128] = gates[i * len(gates) // j].astype(BF16)
                    piece(*work.pop(0))
                gates.clear()
        assert not work and not st
        r = lax.broadcasted_iota(jnp.int32, (64, 128), 0)
        c = lax.broadcasted_iota(jnp.int32, (64, 128), 1)
        msk = (r // 16) == (c % 4)
        for g in range(8):
            z_s[g] = zs[g]
            kvT[g] = _pk(jnp.where(msk, kvs[g], 0.0))
        wait(7)

    def phase2(half):
        base = pl.multiple_of(half * (S // 2), S // 2)
        gbase = half * (S // 256)
        HM = TM // 2
        last = S // (2 * TM) - 1

        def row(u, i=0):
            return pl.multiple_of(base + (u * TM + i * HM), HM)

        def w2_part(u, i):
            r0 = row(u, i)
            hsft = jnp.concatenate(
                [h_scr[g, pl.ds(r0 + 8 + sh, HM), :] for g, sh in enumerate((-1, 1, -2, 2))],
                axis=1)
            a7 = lhs7(hsft)
            hs = _merge_rows(*sw_mm(a7, R2, Q2, wf_v))
            x1 = xr(r0, HM).astype(F32) + hs
            m, r = _ln_stats(x1)
            return x1, (x1 - m) * r

        def q_part(u, i):
            qT = _nt(_up(wqT[...]), xr(row(u, i), HM))
            gate = g_s[gbase + 2 * u + i]
            fqs = []
            for g, pg in enumerate(_groups(qT)):
                ep, en, sp, sn = _exps(pg)
                z = zb[g]
                ap = _fold4(jnp.sum(ep * z[0:64].reshape(8, 8, HM), axis=0), jnp.add)
                an = _fold4(jnp.sum(en * z[64:128].reshape(8, 8, HM), axis=0), jnp.add)
                rd = gate * _rcp(ap * sn + an * sp + 1e-6 * (sp * sn))
                fqs.append(jnp.concatenate([(ep * (sn * rd)[None]).reshape(64, HM),
                                            (en * (sp * rd)[None]).reshape(64, HM)], axis=0))
            return fqs

        def emit(r0, n, val):
            idx = pl.ds(r0, n)
            o_v[idx, :] = val.astype(BF16)
            cp(o_v.at[idx], out_hbm.at[idx], OSEM).start()

        def out_stage(u, oT, b):
            a = [w.astype(BF16).T
                 for w in _wino_a(oT[:HD, :HM], oT[HD:, :HM], oT[:HD, HM:], oT[HD:, HM:])]
            if u == last:
                a0 = 0
                for n in TAIL:
                    ac = [w[a0:a0 + n] for w in a]
                    if a0 + n == HM:
                        a21 = oT[:HD, HM:].astype(BF16).T[a0:a0 + n]
                        y = (_nn(jnp.concatenate([ac[0], a21], axis=0), wf_v[RO:RO + HD, :])
                             + _nn(jnp.concatenate([ac[1], ac[3]], axis=0),
                                   wf_v[RO + HD:RO + D, :]))
                        top, bot = y[:n], y[n:]
                    else:
                        top, bot = sw_mm(ac, RO, QO, wf_v)
                    emit(row(u) + a0, n, top + b[a0:a0 + n])
                    emit(row(u) + HM + a0, n, bot + b[HM + a0:HM + a0 + n])
                    a0 += n
            else:
                res = sw_mm(a, RO, QO, wf_v)
                emit(row(u), TM, jnp.concatenate(res, axis=0) + b)

        st = {}

        def w3_gen(u):
            ln = jnp.concatenate([st.pop(('ln0', u)), st.pop(('ln1', u))], axis=0)
            a = lhs7(ln)
            outs = []
            for n in range(HF // 128):
                lo_ = pl.ds(R3 + n * 128, 128)
                hi_ = pl.ds(R3 + HF + n * 128, 128)
                ta_ = pl.ds(Q3 + n * 128, 128)
                tb_ = pl.ds(Q3 + HF + n * 128, 128)
                c = _wino_c(_nt, a, wf_v[lo_, 0:HD], wf_v[lo_, HD:D], wf_v[hi_, HD:D],
                            wf_v[ta_, 0:HD], wf_v[ta_, HD:D], wf_v[tb_, 0:HD], wf_v[tb_, HD:D])
                outs.append(_wino_a(*[_gelu(t) for t in c]))
                if n in (1, 3):
                    yield
            hr = _gelu(_nt(wf_v[R3 + FM:R3 + Fd, :], ln.astype(BF16))).astype(BF16)
            st['h3', u] = [jnp.concatenate([o[i] for o in outs], axis=1).astype(BF16)
                           for i in range(7)]
            st['hr', u] = hr.T
            yield

        def w4_gen(u):
            a11, a12, s4, a22, s1, s2, s3 = st['h3', u]
            ht, hb = _split_rows(st['hr', u])
            res = []
            for n in range(2):
                l_, r_ = pl.ds(n * 128, 128), pl.ds(HD + n * 128, 128)
                lo_, hi_ = pl.ds(R4, HF), pl.ds(R4 + HF, HF)
                ta_, tb_ = pl.ds(Q4, HF), pl.ds(Q4 + HF, HF)
                tail = pl.ds(R4 + FM, Fd - FM)
                p1 = _nn(a11, wf_v[lo_, l_])
                u2 = p1 + _nn(s2, wf_v[ta_, r_])
                c11 = p1 + _nn(a12, wf_v[hi_, l_]) + _nn(ht, wf_v[tail, l_])
                yield
                u3 = u2 + _nn(s3, wf_v[tb_, l_])
                p5 = _nn(s1, wf_v[ta_, l_])
                c12 = u2 + p5 + _nn(s4, wf_v[hi_, r_]) + _nn(ht, wf_v[tail, r_])
                yield
                c22 = u3 + p5 + _nn(hb, wf_v[tail, r_])
                c21 = u3 - _nn(a22, wf_v[tb_, r_]) + _nn(hb, wf_v[tail, l_])
                res.append((c11, c12, c21, c22))
                if n == 1:
                    st['y', u] = res
                yield

        for g in range(8):
            zb[g] = jnp.broadcast_to(jnp.sum(z_s[g], axis=1, keepdims=True), (128, 128))
        for op in SEQ2.split():
            c, u = op[0], int(op[1])
            if c == 'b':
                i = 0 if ('x10', u) not in st else 1
                st['x1%d' % i, u], st['ln%d' % i, u] = w2_part(u, i)
            elif c == 'q':
                i = 0 if ('q0', u) not in st else 1
                st['q%d' % i, u] = q_part(u, i)
            elif c in 'ce':
                if (c, u) not in st:
                    st[c, u] = w3_gen(u) if c == 'c' else w4_gen(u)
                next(st[c, u])
            elif c == 'N':
                fq = [jnp.concatenate([a_, b_], axis=1).astype(BF16)
                      for a_, b_ in zip(st.pop(('q0', u)), st.pop(('q1', u)))]
                o = {g: _nn(_up(kvT[g]), fq[g]) for g in (0, 4, 1, 5, 2, 6, 3, 7)}
                st['oT', u] = jnp.concatenate([o[g] for g in range(8)], axis=0)
            elif c == 'O':
                y = _merge_rows(*sw_join(st.pop(('y', u))))
                b = jnp.concatenate([st.pop(('x10', u)), st.pop(('x11', u))], axis=0) + y
                b = b * jnp.concatenate([ng_s[pl.ds(row(u), TM), :]] * 4, axis=1)
                out_stage(u, st.pop(('oT', u)), b)

    def main(i, carry):
        pl.when(i == 0)(lambda: phase1(i))
        pl.when(i > 0)(lambda: phase2(i - 1))
        return carry

    lax.fori_loop(0, 3, main, 0)
    cp(o_v, out_hbm, OSEM).wait()


@jax.jit
def pallas_gated_mix__linear_kernel_hedgehog__mixer_s_mlp__prompt_kernel(
    A_x: jax.Array,
    A_wqkv: jax.Array,
    A_w_phi: jax.Array,
    A_wo: jax.Array,
    B_x: jax.Array,
    B_w1: jax.Array,
    B_w2: jax.Array,
    B_w3: jax.Array,
    B_w4: jax.Array,
    gate_w: jax.Array,
):
    B, S, D = A_x.shape
    Fd = B_w3.shape[1]
    assert (B, S, D, Fd) == (1, 8 * TM, 512, 1376) and A_w_phi.shape == (32, 16, 16)
    FM = (Fd // 256) * 256
    x2 = A_x.reshape(S, D)
    wphi2 = A_w_phi.transpose(1, 2, 0).reshape(256, 32)
    gw2 = gate_w.reshape(4, 128)
    w3t = B_w3.T
    anyspec = pl.BlockSpec(memory_space=pl.ANY)
    out = pl.pallas_call(
        functools.partial(_kernel, S=S, D=D, Fd=Fd),
        in_specs=[anyspec] * 9,
        out_specs=anyspec,
        out_shape=jax.ShapeDtypeStruct((S, D), A_x.dtype),
        scratch_shapes=[
            pltpu.VMEM((S, D), BF16),
            pltpu.VMEM((D, 3 * D), BF16),
            pltpu.VMEM((256, 32), BF16),
            pltpu.VMEM((2 * D, D), BF16),
            pltpu.VMEM((4, D // 4, D // 2), U32),
            pltpu.VMEM((2 * Fd + 2 * FM + 4 * D + 16, D), BF16),
            pltpu.VMEM((4, 128), BF16),
            pltpu.VMEM((S, D), BF16),
            pltpu.VMEM((D, 128), BF16),
            pltpu.VMEM((248, D), U32),
            pltpu.VMEM((D // 2, D), U32),
            pltpu.VMEM((240, D), U32),
            pltpu.VMEM((4, S + 16, 128), F32),
            pltpu.VMEM((8, 32, 128), U32),
            pltpu.VMEM((8, 128, 128), F32),
            pltpu.VMEM((8, 128, 128), F32),
            pltpu.VMEM((S // 128, 8, 128), F32),
            pltpu.VMEM((S, 128), F32),
            pltpu.SemaphoreType.DMA((9,)),
        ],
        compiler_params=pltpu.CompilerParams(vmem_limit_bytes=100 * 1024 * 1024,
                                             disable_bounds_checks=True,
                                             disable_semaphore_checks=True),
    )(x2, A_wqkv, wphi2, A_wo, B_w1, B_w2, w3t, B_w4, gw2)
    return out.reshape(B, S, D)
```

```python
import functools

import jax
import jax.numpy as jnp
from jax import lax
import jax.experimental.pallas as pl
import jax.experimental.pallas.tpu as pltpu

F32 = jnp.float32
BF16 = jnp.bfloat16
U32 = jnp.uint32
TM = 256
IL = 16
RB = 8
GROUPS = (('x1', 'v'), ('x2', 'x3', 'x4', '4'), ('x5', 'x6', 'x7', 'q', '3', '2', 'o'))
SEQ1 = ('W4 p1 K1 K1 T h1 h1 V0 v1 a0 a0 v1 a1 a1 '
        'W5 K2 K2 v2 v2 h2 c32 a2 a2 h2 K3 K3 v3 v3 h3 h3 c32 a3 a3 h4 h4 '
        'W6 Q K4 K4 v4 v4 a4 c28 a4 K5 K5 v5 c36 v5 h5 h5 K6 a5 a5 K6 v6 c48 v6 h6 '
        'K7 h6 a6 a6 K7 c48 v7 v7 h7 h7 a7 a7')
SEQ2 = ('b0 b0 q0 b1 c0 c0 c0 e0 e0 b1 e0 c1 q0 e0 N0 e0 c1 b2 c1 e0 b2 O0 '
        'e1 q1 c2 c2 q1 e1 e1 e1 N1 e1 b3 e1 O1 b3 c2 e2 q2 q2 e2 e2 c3 e2 N2 e2 c3 e2 c3 O2 '
        'q3 e3 e3 q3 e3 N3 e3 e3 e3 O3')
TAIL = (64, 48, 16)
NT_DIMS = (((1,), (1,)), ((), ()))
GC = 0.7978845608028654
LOG2E = 1.4426950408889634


def _gelu(x):
    return (0.5 * x) * (1.0 + jnp.tanh(x * (GC + (GC * 0.044715) * (x * x))))


def _rcp(x):
    return pl.reciprocal(x, approx=False, full_range=False)


def _ln_stats(xf):
    m = jnp.mean(xf, axis=-1, keepdims=True)
    v = jnp.maximum(jnp.mean(xf * xf, axis=-1, keepdims=True) - m * m, 0.0)
    return m, lax.rsqrt(v + 1e-5)


def _pk(x):
    return pltpu.bitcast(x.astype(BF16), U32)


def _up(x):
    return pltpu.bitcast(x, BF16)


def _nt(a, b):
    return lax.dot_general(a, b, NT_DIMS, preferred_element_type=F32)


def _nn(a, b):
    return jnp.dot(a, b, preferred_element_type=F32)


def _fold4(a, op):
    return op(a, pltpu.roll(a, 4, 0))


def _exps(p):
    p3 = p.reshape(8, 8, p.shape[1])
    mx = _fold4(jnp.max(p3, axis=0), jnp.maximum)
    mn = _fold4(jnp.min(p3, axis=0), jnp.minimum)
    ep = jnp.exp2(p3 - mx[None])
    en = jnp.exp2(mn[None] - p3)
    sp = _fold4(jnp.sum(ep, axis=0), jnp.add)
    sn = _fold4(jnp.sum(en, axis=0), jnp.add)
    return ep, en, sp, sn


def _groups(pT):
    lo = lax.broadcasted_iota(jnp.int32, (8, pT.shape[1]), 0) < 4
    for hg in range(4):
        blk = pT[hg * 120:(hg + 1) * 120]
        mid = blk[0:8]
        yield jnp.concatenate([jnp.where(lo, mid, 0.0), blk[8:64]], axis=0)
        yield jnp.concatenate([jnp.where(lo, 0.0, mid), blk[64:120]], axis=0)


def _wino_a(a11, a12, a21, a22):
    s1 = a21 + a22
    s2 = s1 - a11
    s3 = a11 - a21
    s4 = a12 - s2
    return a11, a12, s4, a22, s1, s2, s3


def _wino_b(b11, b12, b21, b22):
    t1 = b12 - b11
    t2 = b22 - t1
    t3 = b22 - b12
    t4 = t2 - b21
    return t1, t2, t3, t4


def _wino_2(mm, a, b11, b21, b22, t1, t2, t3, t4):
    a11, a12, s4, a22, s1, s2, s3 = a
    p1 = mm(a11, b11)
    u2 = p1 + mm(s2, t2)
    c11 = p1 + mm(a12, b21)
    u3 = u2 + mm(s3, t3)
    yield u2, u3
    p5 = mm(s1, t1)
    c12 = u2 + p5 + mm(s4, b22)
    c22 = u3 + p5
    c21 = u3 - mm(a22, t4)
    yield c11, c12, c21, c22


def _wino_c(*args):
    return list(_wino_2(*args))[-1]


def _split_rows(a):
    m, n = a.shape
    a4 = a.reshape(m // (2 * IL), 2, IL, n)
    return a4[:, 0].reshape(m // 2, n), a4[:, 1].reshape(m // 2, n)


def _merge_rows(top, bot):
    h, n = top.shape
    return jnp.stack([top.reshape(h // IL, IL, n), bot.reshape(h // IL, IL, n)],
                     axis=1).reshape(2 * h, n)


def _kernel(x_hbm, wqkv_hbm, wphi_hbm, wo_hbm, w1_hbm, w2_hbm, w3t_hbm, w4_hbm, gw_hbm,
            out_hbm,
            x_v, wqkv_v, wphi_v, w1_v, sv_s, wf_v, gw_v, o_v,
            p_s, wkT, wvT, wqT, h_scr, kvT, zb, z_s, g_s, ng_s, sems,
            *, S, D, Fd):
    FM = (Fd // 256) * 256
    HF, HD = FM // 2, D // 2
    R3, R4, R2, RO = 0, Fd, 2 * Fd, 2 * Fd + D
    Q3 = 2 * Fd + 2 * D
    Q4, Q2, QO = Q3 + FM, Q3 + 2 * FM, Q3 + 2 * FM + D
    DUM = QO + D
    OSEM = 8

    def cp(src, dst, k):
        return pltpu.make_async_copy(src, dst, sems.at[k])

    def named(items, k):
        out = []
        xs = [int(i[1:]) for i in items if i[0] == 'x']
        for it in items:
            if it[0] == 'x':
                if int(it[1:]) == xs[0]:
                    r = pl.ds(xs[0] * TM, len(xs) * TM)
                    out.append(cp(x_hbm.at[r], x_v.at[r], k))
            elif it in 'qkv':
                c = (slice(None), pl.ds('qkv'.index(it) * D, D))
                out.append(cp(wqkv_hbm.at[c], wqkv_v.at[c], k))
            else:
                src, row, n = {'3': (w3t_hbm.at[pl.ds(0, FM)], R3, FM),
                               '4': (w4_hbm.at[pl.ds(0, FM)], R4, FM),
                               '2': (w2_hbm, R2, D), 'o': (wo_hbm, RO, D)}[it]
                out.append(cp(src, wf_v.at[pl.ds(row, n)], k))
        return out

    tail_rows = pl.ds(FM, Fd - FM)
    copies = [[cp(wphi_hbm, wphi_v, 0), cp(gw_hbm, gw_v, 0)], named(['k'], 1), named(['x0'], 2),
              [cp(w1_hbm, w1_v.at[pl.ds(0, D)], 3)]]
    copies += [named(g, 4 + i) for i, g in enumerate(GROUPS)]
    copies += [[cp(w3t_hbm.at[tail_rows], wf_v.at[pl.ds(R3 + FM, Fd - FM)], 7),
                cp(w4_hbm.at[tail_rows], wf_v.at[pl.ds(R4 + FM, Fd - FM)], 7)]]
    for grp in copies:
        for c in grp:
            c.start()

    def wait(k):
        for c in copies[k]:
            c.wait()

    h_scr[:, 0:8, :] = jnp.zeros((4, 8, 128), F32)
    h_scr[:, S + 8:S + 16, :] = jnp.zeros((4, 8, 128), F32)

    def row_info(n):
        rr = lax.broadcasted_iota(jnp.int32, (D, n), 0)
        hg = rr // 128
        rr = rr % 128
        f = jnp.where(rr < 16, rr // 8, jnp.where(rr < 72, rr // 4 - 2, rr // 4 - 16))
        hl8 = jnp.where(rr < 16, rr % 8, jnp.where(rr < 72, rr % 4, 4 + rr % 4))
        return hg, f, hl8, lax.broadcasted_iota(jnp.int32, (D, n), 1)

    def fold(col0):
        lo = lax.broadcasted_iota(jnp.int32, (8, D), 0) < 4
        outs = []
        for hg in range(4):
            W = wqkv_v[:, col0 + hg * 128: col0 + (hg + 1) * 128]
            WT = _nt(p_s[hg * 128:(hg + 1) * 128, :], W) * LOG2E
            ref = WT[0:8]
            rot = pltpu.roll(ref, 4, 0)
            outs.append(WT[8:16] - ref)
            outs.append((WT[16:72].reshape(7, 8, D) - jnp.where(lo, ref, rot)[None]).reshape(56, D))
            outs.append((WT[72:128].reshape(7, 8, D) - jnp.where(lo, rot, ref)[None]).reshape(56, D))
        return _pk(jnp.concatenate(outs, axis=0))

    def xr(r0, n):
        return x_v[pl.ds(r0, n), :]

    def sw_mm(a, src, dst, bank):
        lo_, hi_ = pl.ds(src, HD), pl.ds(src + HD, HD)
        ta_, tb_ = pl.ds(dst, HD), pl.ds(dst + HD, HD)
        return sw_join([_wino_c(_nn, a, bank[lo_, 0:HD], bank[hi_, 0:HD], bank[hi_, HD:D],
                                bank[ta_, 0:HD], bank[ta_, HD:D], bank[tb_, 0:HD],
                                bank[tb_, HD:D])])

    def sw_join(cs_):
        top = jnp.concatenate([c[0] for c in cs_] + [c[1] for c in cs_], axis=1)
        bot = jnp.concatenate([c[2] for c in cs_] + [c[3] for c in cs_], axis=1)
        return top, bot

    def lhs7(a):
        top, bot = _split_rows(a)
        return [u.astype(BF16)
                for u in _wino_a(top[:, :HD], top[:, HD:], bot[:, :HD], bot[:, HD:])]

    def phase1(step):
        wait(0)
        hg_, f_, hl8_, c = row_info(32)
        A = ((hg_ * 8 + hl8_) == c).astype(BF16)
        T1_ = _nt(A, wphi_v[...])
        hg_, f_, hl8_, c = row_info(256)
        T2_ = jnp.where(f_ == (c % 16), T1_, 0.0).astype(BF16)
        r = lax.broadcasted_iota(jnp.int32, (256, 128), 0)
        c = lax.broadcasted_iota(jnp.int32, (256, 128), 1)
        Bm = ((r // 16) == (c % 16)).astype(BF16)
        P = _nn(T2_, Bm)
        hg_, f_, hl8_, c = row_info(128)
        p_s[...] = jnp.where(hl8_ == (c // 16), P, 0.0).astype(BF16)
        gw = gw_v[...].astype(F32)
        gwr = jnp.concatenate([gw[g:g + 1] for g in range(4)], axis=1)
        wkT[0:8, :] = _pk(jnp.broadcast_to(gwr, (16, D)))

        zs = [None] * 8
        kvs = [None] * 8
        gates = []
        st = {}
        gens = {}
        off = pl.multiple_of(step * (-HD), 16)

        def k_soft(j, kT):
            gate = jax.nn.sigmoid(kT[0:8])
            for i in range(2):
                g_s[2 * j + i] = gate[:, i * 128:(i + 1) * 128]
            ng_s[pl.ds(j * TM, TM), :] = jnp.concatenate([1.0 - gate] * 16, axis=0).T
            fks = []
            for g, pg in enumerate(_groups(kT[16:496])):
                ep, en, sp, sn = _exps(pg)
                fk = jnp.concatenate([(ep * _rcp(sp)[None]).reshape(64, TM),
                                      (en * _rcp(sn)[None]).reshape(64, TM)], axis=0)
                part = fk[:, 0:128] + fk[:, 128:256]
                zs[g] = part if zs[g] is None else zs[g] + part
                fks.append(fk.astype(BF16))
            return fks

        def v_split(vT):
            return [vT[g * 64:(g + 1) * 64, :].astype(BF16) for g in range(8)]

        def v_sw(j):
            xb = xr(j * TM, TM)
            xf = xb.astype(F32)
            h = TM // 2
            tx = [u.astype(BF16) for u in
                  _wino_b(xf[:h, :HD], xf[h:, :HD], xf[:h, HD:], xf[h:, HD:])]
            q4 = D // 4
            av = (_up(wvT[0:q4, 0:HD]), _up(wvT[0:q4, HD:D]), _up(sv_s[3]),
                  _up(wvT[q4:2 * q4, HD:D]), _up(sv_s[0]), _up(sv_s[1]), _up(sv_s[2]))
            it = _wino_2(_nt, av, xb[:h, :HD], xb[:h, HD:], xb[h:, HD:], *tx)
            gates.extend(a_[r * 8:(r + 1) * 8] for a_ in next(it) for r in range(HD // 8))
            yield
            c11, c12, c21, c22 = next(it)
            st['v', j] = v_split(jnp.concatenate([jnp.concatenate([c11, c12], axis=1),
                                                  jnp.concatenate([c21, c22], axis=1)], axis=0))
            yield

        def k_gen(j):
            ks = []
            for n in range(2):
                ks.append(_nt(_up(wkT[...]), xr(j * TM + n * 128, 128)))
                gates.extend(ks[n][r * 8:(r + 1) * 8] for r in range(62))
                if n == 1:
                    st['f', j] = k_soft(j, jnp.concatenate(ks, axis=1))
                yield

        def a_gen(j):
            fks, vT = st.pop(('f', j)), st.pop(('v', j))
            for g in range(8):
                part = _nt(vT[g], fks[g])
                kvs[g] = part if kvs[g] is None else kvs[g] + part
                if g % 4 == 3:
                    yield

        def h_store(j, g, y):
            h_scr[g, pl.ds(j * TM + 8, TM), :] = _gelu(y)

        def h_sw(j):
            xf = xr(j * TM, TM).astype(F32)
            m_, r_ = _ln_stats(xf)
            a7 = lhs7((xf - m_) * r_)
            it = _wino_2(_nn, a7, w1_v[0:HD, 0:HD], w1_v[HD:D, 0:HD], w1_v[HD:D, HD:D],
                         w1_v[D:D + HD, 0:HD], w1_v[D:D + HD, HD:D],
                         w1_v[D + HD:2 * D, 0:HD], w1_v[D + HD:2 * D, HD:D])
            next(it)
            yield
            y = _merge_rows(*sw_join([next(it)]))
            for g in range(4):
                h_store(j, g, y[:, g * 128:(g + 1) * 128])
            yield

        tab = {'3': (wf_v, R3, Q3, HF, True), '4': (wf_v, R4, Q4, HF, False),
               '2': (wf_v, R2, Q2, HD, False), 'o': (wf_v, RO, QO, HD, False),
               '1': (w1_v, 0, D, HD, False)}

        def piece(key, r0):
            bank, src, dst, H, tr = tab[key]
            lo_ = bank[src + r0:src + r0 + RB, :].astype(F32)
            hi_ = bank[src + H + r0:src + H + r0 + RB, :].astype(F32)
            if tr:
                t1, t2, t3, t4 = _wino_b(lo_[:, :HD], hi_[:, :HD], lo_[:, HD:], hi_[:, HD:])
            else:
                t1, t2, t3, t4 = _wino_b(lo_[:, :HD], lo_[:, HD:], hi_[:, :HD], hi_[:, HD:])
            bank[pl.ds(off + dst + r0, RB), :] = jnp.concatenate([t1, t2], axis=1).astype(BF16)
            bank[pl.ds(off + dst + H + r0, RB), :] = jnp.concatenate([t3, t4], axis=1).astype(BF16)

        work = [(k, r0) for k in '432o' for r0 in range(0, tab[k][3], RB)]

        wait(1)
        wkT[8:248, :] = fold(D)
        wait(2)
        k0 = _nt(_up(wkT[...]), xr(0, TM))
        m0, r0_ = _ln_stats(xr(0, TM).astype(F32))
        st['f', 0] = k_soft(0, k0)
        wait(3)
        cs = jnp.sum(w1_v[0:D, :].astype(F32), axis=0, keepdims=True)
        y = (_nn(xr(0, TM), w1_v[0:D, :]) - m0 * cs) * r0_
        for g in range(4):
            h_store(0, g, y[:, g * 128:(g + 1) * 128])
        for op in SEQ1.split():
            c, j = op[0], int(op[1:] or 0)
            if c == 'W':
                wait(j)
                gates.clear()
            elif c == 'p':
                for r0 in range(0, HD, RB):
                    piece('1', r0)
            elif c in 'Kvha':
                if op not in gens:
                    gens[op] = {'K': k_gen, 'v': v_sw, 'h': h_sw, 'a': a_gen}[c](j)
                next(gens[op])
            elif c == 'T':
                wvt = wqkv_v[:, 2 * D:3 * D].T
                wvT[...] = _pk(wvt)
                wf32 = wvt.astype(F32)
                _, _, s4, _, s1, s2, s3 = _wino_a(wf32[:HD, :HD], wf32[:HD, HD:],
                                                  wf32[HD:, :HD], wf32[HD:, HD:])
                for i, u in enumerate((s1, s2, s3, s4)):
                    sv_s[i] = _pk(u)
            elif c == 'V':
                st['v', j] = v_split(_nt(_up(wvT[...]), xr(j * TM, TM)))
            elif c == 'Q':
                wqT[...] = fold(0)
            elif c == 'c':
                for i in range(j):
                    wf_v[pl.ds(off + DUM, 8), 0:128] = gates[i * len(gates) // j].astype(BF16)
                    piece(*work.pop(0))
                gates.clear()
        assert not work and not st
        r = lax.broadcasted_iota(jnp.int32, (64, 128), 0)
        c = lax.broadcasted_iota(jnp.int32, (64, 128), 1)
        msk = (r // 16) == (c % 4)
        for g in range(8):
            z_s[g] = zs[g]
            kvT[g] = _pk(jnp.where(msk, kvs[g], 0.0))
        wait(7)

    def phase2(half):
        base = pl.multiple_of(half * (S // 2), S // 2)
        gbase = half * (S // 256)
        HM = TM // 2
        last = S // (2 * TM) - 1

        def row(u, i=0):
            return pl.multiple_of(base + (u * TM + i * HM), HM)

        def w2_part(u, i):
            r0 = row(u, i)
            hsft = jnp.concatenate(
                [h_scr[g, pl.ds(r0 + 8 + sh, HM), :] for g, sh in enumerate((-1, 1, -2, 2))],
                axis=1)
            a7 = lhs7(hsft)
            hs = _merge_rows(*sw_mm(a7, R2, Q2, wf_v))
            x1 = xr(r0, HM).astype(F32) + hs
            m, r = _ln_stats(x1)
            return x1, (x1 - m) * r

        def q_part(u, i):
            qT = _nt(_up(wqT[...]), xr(row(u, i), HM))
            gate = g_s[gbase + 2 * u + i]
            fqs = []
            for g, pg in enumerate(_groups(qT)):
                ep, en, sp, sn = _exps(pg)
                z = zb[g]
                ap = _fold4(jnp.sum(ep * z[0:64].reshape(8, 8, HM), axis=0), jnp.add)
                an = _fold4(jnp.sum(en * z[64:128].reshape(8, 8, HM), axis=0), jnp.add)
                rd = gate * _rcp(ap * sn + an * sp + 1e-6 * (sp * sn))
                fqs.append(jnp.concatenate([(ep * (sn * rd)[None]).reshape(64, HM),
                                            (en * (sp * rd)[None]).reshape(64, HM)], axis=0))
            return fqs

        def emit(r0, n, val):
            idx = pl.ds(r0, n)
            o_v[idx, :] = val.astype(BF16)
            cp(o_v.at[idx], out_hbm.at[idx], OSEM).start()

        def out_stage(u, oT, b):
            a = [w.astype(BF16).T
                 for w in _wino_a(oT[:HD, :HM], oT[HD:, :HM], oT[:HD, HM:], oT[HD:, HM:])]
            if u == last:
                a0 = 0
                for n in TAIL:
                    ac = [w[a0:a0 + n] for w in a]
                    if a0 + n == HM:
                        a21 = oT[:HD, HM:].astype(BF16).T[a0:a0 + n]
                        y = (_nn(jnp.concatenate([ac[0], a21], axis=0), wf_v[RO:RO + HD, :])
                             + _nn(jnp.concatenate([ac[1], ac[3]], axis=0),
                                   wf_v[RO + HD:RO + D, :]))
                        top, bot = y[:n], y[n:]
                    else:
                        top, bot = sw_mm(ac, RO, QO, wf_v)
                    emit(row(u) + a0, n, top + b[a0:a0 + n])
                    emit(row(u) + HM + a0, n, bot + b[HM + a0:HM + a0 + n])
                    a0 += n
            else:
                res = sw_mm(a, RO, QO, wf_v)
                emit(row(u), TM, jnp.concatenate(res, axis=0) + b)

        st = {}

        def w3_gen(u):
            ln = jnp.concatenate([st.pop(('ln0', u)), st.pop(('ln1', u))], axis=0)
            a = lhs7(ln)
            outs = []
            for n in range(HF // 128):
                lo_ = pl.ds(R3 + n * 128, 128)
                hi_ = pl.ds(R3 + HF + n * 128, 128)
                ta_ = pl.ds(Q3 + n * 128, 128)
                tb_ = pl.ds(Q3 + HF + n * 128, 128)
                c = _wino_c(_nt, a, wf_v[lo_, 0:HD], wf_v[lo_, HD:D], wf_v[hi_, HD:D],
                            wf_v[ta_, 0:HD], wf_v[ta_, HD:D], wf_v[tb_, 0:HD], wf_v[tb_, HD:D])
                outs.append(_wino_a(*[_gelu(t) for t in c]))
                if n in (1, 3):
                    yield
            hr = _gelu(_nt(wf_v[R3 + FM:R3 + Fd, :], ln.astype(BF16))).astype(BF16)
            st['h3', u] = [jnp.concatenate([o[i] for o in outs], axis=1).astype(BF16)
                           for i in range(7)]
            st['hr', u] = hr.T
            yield

        def w4_gen(u):
            a11, a12, s4, a22, s1, s2, s3 = st['h3', u]
            ht, hb = _split_rows(st['hr', u])
            res = []
            for n in range(2):
                l_, r_ = pl.ds(n * 128, 128), pl.ds(HD + n * 128, 128)
                lo_, hi_ = pl.ds(R4, HF), pl.ds(R4 + HF, HF)
                ta_, tb_ = pl.ds(Q4, HF), pl.ds(Q4 + HF, HF)
                tail = pl.ds(R4 + FM, Fd - FM)
                p1 = _nn(a11, wf_v[lo_, l_])
                u2 = p1 + _nn(s2, wf_v[ta_, r_])
                c11 = p1 + _nn(a12, wf_v[hi_, l_]) + _nn(ht, wf_v[tail, l_])
                yield
                u3 = u2 + _nn(s3, wf_v[tb_, l_])
                p5 = _nn(s1, wf_v[ta_, l_])
                c12 = u2 + p5 + _nn(s4, wf_v[hi_, r_]) + _nn(ht, wf_v[tail, r_])
                yield
                c22 = u3 + p5 + _nn(hb, wf_v[tail, r_])
                c21 = u3 - _nn(a22, wf_v[tb_, r_]) + _nn(hb, wf_v[tail, l_])
                res.append((c11, c12, c21, c22))
                if n == 1:
                    st['y', u] = res
                yield

        for g in range(8):
            zb[g] = jnp.broadcast_to(jnp.sum(z_s[g], axis=1, keepdims=True), (128, 128))
        for op in SEQ2.split():
            c, u = op[0], int(op[1])
            if c == 'b':
                i = 0 if ('x10', u) not in st else 1
                st['x1%d' % i, u], st['ln%d' % i, u] = w2_part(u, i)
            elif c == 'q':
                i = 0 if ('q0', u) not in st else 1
                st['q%d' % i, u] = q_part(u, i)
            elif c in 'ce':
                if (c, u) not in st:
                    st[c, u] = w3_gen(u) if c == 'c' else w4_gen(u)
                next(st[c, u])
            elif c == 'N':
                fq = [jnp.concatenate([a_, b_], axis=1).astype(BF16)
                      for a_, b_ in zip(st.pop(('q0', u)), st.pop(('q1', u)))]
                o = {g: _nn(_up(kvT[g]), fq[g]) for g in (0, 4, 1, 5, 2, 6, 3, 7)}
                st['oT', u] = jnp.concatenate([o[g] for g in range(8)], axis=0)
            elif c == 'O':
                y = _merge_rows(*sw_join(st.pop(('y', u))))
                b = jnp.concatenate([st.pop(('x10', u)), st.pop(('x11', u))], axis=0) + y
                b = b * jnp.concatenate([ng_s[pl.ds(row(u), TM), :]] * 4, axis=1)
                out_stage(u, st.pop(('oT', u)), b)

    def main(i, carry):
        pl.when(i == 0)(lambda: phase1(i))
        pl.when(i > 0)(lambda: phase2(i - 1))
        return carry

    lax.fori_loop(0, 3, main, 0)
    cp(o_v, out_hbm, OSEM).wait()


@jax.jit
def pallas_gated_mix__linear_kernel_hedgehog__mixer_s_mlp__prompt_kernel(
    A_x: jax.Array,
    A_wqkv: jax.Array,
    A_w_phi: jax.Array,
    A_wo: jax.Array,
    B_x: jax.Array,
    B_w1: jax.Array,
    B_w2: jax.Array,
    B_w3: jax.Array,
    B_w4: jax.Array,
    gate_w: jax.Array,
):
    B, S, D = A_x.shape
    Fd = B_w3.shape[1]
    assert (B, S, D, Fd) == (1, 8 * TM, 512, 1376) and A_w_phi.shape == (32, 16, 16)
    FM = (Fd // 256) * 256
    x2 = A_x.reshape(S, D)
    wphi2 = A_w_phi.transpose(1, 2, 0).reshape(256, 32)
    gw2 = gate_w.reshape(4, 128)
    w3t = B_w3.T
    anyspec = pl.BlockSpec(memory_space=pl.ANY)
    out = pl.pallas_call(
        functools.partial(_kernel, S=S, D=D, Fd=Fd),
        in_specs=[anyspec] * 9,
        out_specs=anyspec,
        out_shape=jax.ShapeDtypeStruct((S, D), A_x.dtype),
        scratch_shapes=[
            pltpu.VMEM((S, D), BF16),
            pltpu.VMEM((D, 3 * D), BF16),
            pltpu.VMEM((256, 32), BF16),
            pltpu.VMEM((2 * D, D), BF16),
            pltpu.VMEM((4, D // 4, D // 2), U32),
            pltpu.VMEM((2 * Fd + 2 * FM + 4 * D + 16, D), BF16),
            pltpu.VMEM((4, 128), BF16),
            pltpu.VMEM((S, D), BF16),
            pltpu.VMEM((D, 128), BF16),
            pltpu.VMEM((248, D), U32),
            pltpu.VMEM((D // 2, D), U32),
            pltpu.VMEM((240, D), U32),
            pltpu.VMEM((4, S + 16, 128), F32),
            pltpu.VMEM((8, 32, 128), U32),
            pltpu.VMEM((8, 128, 128), F32),
            pltpu.VMEM((8, 128, 128), F32),
            pltpu.VMEM((S // 128, 8, 128), F32),
            pltpu.VMEM((S, 128), F32),
            pltpu.SemaphoreType.DMA((9,)),
        ],
        compiler_params=pltpu.CompilerParams(vmem_limit_bytes=100 * 1024 * 1024,
                                             disable_bounds_checks=True,
                                             disable_semaphore_checks=True),
    )(x2, A_wqkv, wphi2, A_wo, B_w1, B_w2, w3t, B_w4, gw2)
    return out.reshape(B, S, D)
```
